```python
import jax
import jax.numpy as jnp

def _softmax(x, axis=-1):
    return jax.nn.softmax(x, axis=axis)

def _gelu(x):
    return jax.nn.gelu(x, approximate=True)

def _silu(x):
    return jax.nn.silu(x)

def _sigmoid(x):
    return jax.nn.sigmoid(x)

def _layernorm(x, axis=-1, eps=1e-05):
    m = jnp.mean(x, axis=axis, keepdims=True)
    v = jnp.var(x, axis=axis, keepdims=True)
    return (x - m) / jnp.sqrt(v + eps)

def _scatter_add(tgt, idx, src, axis=0):
    return tgt.at[idx].add(src)

def _segment_sum(src, seg, n):
    return jax.ops.segment_sum(src, seg, n)

class _Rng:

    def __init__(self, key):
        self._k = key

    def _next(self):
        self._k, sub = jax.random.split(self._k)
        return sub

    def normal(self, shape):
        return jax.random.normal(self._next(), shape, dtype=jnp.bfloat16)

    def randint(self, lo, hi, shape):
        return jax.random.randint(self._next(), shape, lo, hi, dtype=jnp.int32)

    def uniform(self, shape, lo=0.0, hi=1.0):
        return jax.random.uniform(self._next(), shape, jnp.bfloat16, lo, hi)

    def permutation(self, n):
        return jax.random.permutation(self._next(), n)
kernel_name = 'adaLN_cond__sliding_local_dilated__glu_gated_bilinear__prompt'

def setup_inputs():
    _rng = _Rng(jax.random.key(int.from_bytes(__import__("os").urandom(4), "little")))
    _w = lambda a: (lambda t: t.astype(jnp.bfloat16) if jnp.issubdtype(t.dtype, jnp.floating) else t)(jnp.asarray(a))

    def _A_setup():
        B, S, D = (1, 2048, 576)
        return {'x': _w((lambda *s: _rng.normal(s) * 0.05)(B, S, D)), 'wqkv': _w((lambda *s: _rng.normal(s) * 0.05)(D, 3 * D)), 'wo': _w((lambda *s: _rng.normal(s) * 0.05)(D, D))}
    _A_in = _A_setup()

    def _B_setup():
        B, S, D, F = (1, 2048, 576, 4608)
        return {'x': _w((lambda *s: _rng.normal(s) * 0.05)(B, S, D)), 'w_gate': _w((lambda *s: _rng.normal(s) * 0.05)(D, F) * D ** (-0.5)), 'w_up': _w((lambda *s: _rng.normal(s) * 0.05)(D, F) * D ** (-0.5)), 'w_down': _w((lambda *s: _rng.normal(s) * 0.05)(F, D) * F ** (-0.5))}
    _B_in = _B_setup()
    return {'A_x': _A_in['x'], 'A_wqkv': _A_in['wqkv'], 'A_wo': _A_in['wo'], 'B_x': _B_in['x'], 'B_w_gate': _B_in['w_gate'], 'B_w_up': _B_in['w_up'], 'B_w_down': _B_in['w_down'], 'c': _w((lambda *s: _rng.normal(s) * 0.05)(1, 576)), 'w_mod': _w((lambda *s: _rng.normal(s) * 0.05)(576, 6 * 576) * 576 ** (-0.5))}

def reference(A_x, A_wqkv, A_wo, B_x, B_w_gate, B_w_up, B_w_down, c, w_mod):

    def _A_ref(x, wqkv, wo):
        B, S, D = x.shape
        H = 32
        Dh = D // H
        W, dil = (8, 2)
        qkv = (lambda x, *d: x.transpose(*d))((x @ wqkv).reshape(B, S, 3, H, Dh), 2, 0, 3, 1, 4)
        q, k, v = (qkv[0], qkv[1], qkv[2])
        scale = Dh ** (-0.5)
        pos = jnp.arange(S)
        off = jnp.arange(W) * dil
        idx = pos[:, None] - off[None, :]
        mask = idx >= 0
        idx_c = jnp.where(mask, idx, 0).reshape(-1)
        kg = k[:, :, idx_c, :].reshape(B, H, S, W, Dh)
        vg = v[:, :, idx_c, :].reshape(B, H, S, W, Dh)
        logits = jnp.einsum('bhsd,bhswd->bhsw', q, kg) * scale
        logits = jnp.where(mask[None, None, :, :], logits, -1000000000.0)
        attn = _softmax(logits, axis=-1)
        o = jnp.einsum('bhsw,bhswd->bhsd', attn, vg)
        return (lambda x, *d: x.transpose(*d))(o, 0, 2, 1, 3).reshape(B, S, D) @ wo

    def _B_ref(x, w_gate, w_up, w_down):
        g = jnp.einsum('bsd,df->bsf', x, w_gate)
        u = jnp.einsum('bsd,df->bsf', x, w_up)
        h = g * u
        return jnp.einsum('bsf,fd->bsd', h, w_down)
    x = A_x
    mod = (_silu(c) @ w_mod).reshape(c.shape[0], 6, 1, -1)
    sa, ca, ga, sb, cb, gb = (mod[:, 0].copy(), mod[:, 1].copy(), mod[:, 2].copy(), mod[:, 3].copy(), mod[:, 4].copy(), mod[:, 5].copy())
    h = _layernorm(x, axis=-1) * (1 + ca) + sa
    x = x + ga * _A_ref(h, A_wqkv, A_wo)
    h = _layernorm(x, axis=-1) * (1 + cb) + sb
    x = x + gb * _B_ref(h, B_w_gate, B_w_up, B_w_down)
    return x
```

```python
import functools, contextlib
import jax, jax.numpy as jnp, numpy as np
from jax import lax
from jax.experimental import pallas as pl
from jax.experimental.pallas import tpu as pltpu

S, D, H, DH, W, DIL, F = 2048, 576, 32, 18, 8, 2, 4608
EPS = 1e-5
SCALE = DH ** -0.5
NEG = -1000000000.0
LOG2E = 1.4426950408889634
NT = (((1,), (1,)), ((), ()))
f32, bf16, u32 = jnp.float32, jnp.bfloat16, jnp.uint32
KT = [(k, min(128, D - k)) for k in range(0, D, 128)]
P = functools.partial
HALO = 16
RB = 8
QS = [[(0, 4 * t + j) for j in range(4)] for t in range(4)] + [[(0, 16), (0, 17), (2, 16), (2, 17)]]
KS = [[(1, 4 * t + j) for j in range(4)] for t in range(4)] + [[(1, 16), (1, 17), None, None]]
VS = [[(2, 4 * t + j) for j in range(4)] for t in range(4)]
TILES = QS[:4] + KS + VS + QS[4:]
QI, KI, VI = [0, 1, 2, 3, 13], [4, 5, 6, 7, 8], [9, 10, 11, 12, 13]
GROUPS = [(0, 4), (4, 9), (9, 14)]


def pack(x):
    return pltpu.bitcast(x.astype(bf16), u32)


def unpack(w):
    return pltpu.bitcast(w, bf16)


def make(TB=256, FC=1152, name="fused", scopes=False, fpos=(1, 3, 5, 7), la=1, lb=2, chain=3, wo6=1, gt=2, g0=4, glast=2, tok=False, pf='0', grp=GROUPS, order='pre', flags=None):
    NB = S // TB
    NC = F // FC
    NA = TB // RB
    scope = jax.named_scope if scopes else (lambda n: contextlib.nullcontext())

    def kernel(x_hbm, wqkv_hbm, wo_hbm, wg_hbm, wu_hbm, wd_hbm, c_hbm, wmod_hbm, o_hbm,
               x_v, wqkv_v, wo_v, wg_v, wu_v, wd_v, c_v, wmod_v,
               modT, tmp, wqkvT, woT, hA, hB, A, B, o_v, aT, x1T, h2, obuf, zs, sems, osem):
        names = []
        copies = {}
        def add(name, src, dst):
            copies[name] = pltpu.make_async_copy(src, dst, sems.at[len(names)])
            names.append(name)
        def cols(name, src, dst, lo, hi):
            add(name, src.at[:, lo:hi], dst.at[:, lo:hi])
        QKV_CUT = [0, 640, 1152, 3 * D]
        MOD_CUT = [0, 384, 768, 1152, 6 * D]
        add("c", c_hbm, c_v)
        cols("wqkv0", wqkv_hbm, wqkv_v, QKV_CUT[0], QKV_CUT[1])
        add("x0", x_hbm.at[:, 0:TB], x_v.at[0])
        for j in range(3):
            cols("wmod%d" % j, wmod_hbm, wmod_v, MOD_CUT[j], MOD_CUT[j + 1])
        for p in (1, 2):
            cols("wqkv%d" % p, wqkv_hbm, wqkv_v, QKV_CUT[p], QKV_CUT[p + 1])
        add("x1", x_hbm.at[:, TB:2 * TB], x_v.at[1])
        add("wo", wo_hbm, wo_v)
        for b in range(2, NB):
            add("x%d" % b, x_hbm.at[:, b * TB:(b + 1) * TB], x_v.at[b])
        cols("wmod3", wmod_hbm, wmod_v, MOD_CUT[3], MOD_CUT[4])
        add("wg", wg_hbm, wg_v)
        add("wu", wu_hbm, wu_v)
        add("wd", wd_hbm, wd_v)
        for n in names:
            copies[n].start()

        def prep_qkv(p):
            copies["wqkv%d" % p].wait()
            for t, (k0, kw) in enumerate(KT):
                for n0 in range(QKV_CUT[p], QKV_CUT[p + 1], 128):
                    nw = min(128, 3 * D - n0)
                    blk = wqkv_v[k0:k0 + kw, n0:n0 + nw].astype(f32)
                    tmp[t, n0:n0 + nw, 0:kw] = blk.T
            for t, (k0, kw) in enumerate(KT):
                for ti in range(*GROUPS[p]):
                    for j, slot in enumerate(TILES[ti]):
                        r0 = (ti * 128 + j * H) // 2
                        if slot is None:
                            wqkvT[r0:r0 + H // 2, k0:k0 + kw] = jnp.zeros((H // 2, kw), u32)
                        else:
                            rows = tmp[t, pl.ds(slot[0] * D + slot[1], H, stride=DH), :]
                            wqkvT[r0:r0 + H // 2, k0:k0 + kw] = pack(rows[:, 0:kw])

        def prep_wo():
            copies["wo"].wait()
            for t, (n0, nw) in enumerate(KT):
                tmp[t, 0:D, 0:nw] = wo_v[:, n0:n0 + nw].astype(f32)
            for t, (n0, nw) in enumerate(KT):
                for ti in range(5):
                    ds = [4 * ti + j for j in range(4)] if ti < 4 else [None, None, 16, 17]
                    parts = [jnp.zeros((H, nw), f32) if d is None else tmp[t, pl.ds(d, H, stride=DH), :][:, 0:nw] for d in ds]
                    woT[n0 // 2:(n0 + nw) // 2, ti * 128:(ti + 1) * 128] = pack(jnp.concatenate(parts, axis=0).T)

        def mod_cols(j):
            copies["wmod%d" % j].wait()
            n_lo, n_hi = MOD_CUT[j], MOD_CUT[j + 1]
            cf = c_v[...].astype(f32)
            sc = jnp.broadcast_to((cf * jax.nn.sigmoid(cf)).astype(bf16), (16, D))
            m = jnp.dot(sc, wmod_v[:, n_lo:n_hi], preferred_element_type=f32)
            for n0 in range(n_lo, n_hi, 128):
                row = m[0:1, n0 - n_lo:n0 - n_lo + 128]
                col = lax.broadcasted_iota(jnp.int32, (1, 128), 1) + n0
                is_scale = ((col >= D) & (col < 2 * D)) | ((col >= 4 * D) & (col < 5 * D))
                row = jnp.where(is_scale, 1.0 + row, row)
                modT[n0:n0 + 128, :] = jnp.broadcast_to(row, (128, 128)).T

        def mod(i):
            return modT[i * D:(i + 1) * D, :]

        def ln(xf):
            m = jnp.sum(xf, axis=0, keepdims=True) * (1.0 / D)
            d = xf - m
            v = jnp.sum(d * d, axis=0, keepdims=True) * (1.0 / D)
            return d * lax.rsqrt(v + EPS)

        def ln1(b, h):
            for j in range(0, TB, 128):
                y = ln(x_v[b, :, j:j + 128].astype(f32)) * mod(1) + mod(0)
                for k0, kw in KT:
                    h[j // 2:j // 2 + 64, k0:k0 + kw] = pack(y[k0:k0 + kw, :].T)

        def proj(p, h, dst):
            t0, t1 = GROUPS[p]
            y = lax.dot_general(unpack(h[...]), unpack(wqkvT[t0 * 64:t1 * 64, :]), NT, preferred_element_type=f32)
            for t in range(t0, t1):
                dst[t, HALO:HALO + TB, :] = y[:, (t - t0) * 128:(t - t0 + 1) * 128]

        def halo(src, dst):
            for t in range(4, 14):
                dst[t, 0:HALO, :] = src[t, TB:TB + HALO, :]

        def attn(b, buf, masked):
            st = {}
            def rows(r0, t, w):
                r = HALO + r0 - DIL * w
                return buf[t, r:r + RB, :]
            def logits(i):
                r0 = i * RB
                q = [rows(r0, t, 0) for t in QI]
                st[i] = []
                for w in range(W):
                    acc = q[0] * rows(r0, KI[0], w)
                    for t in range(1, 5):
                        acc = acc + q[t] * rows(r0, KI[t], w)
                    st[i].append(acc)
            def softmax(i):
                r0 = i * RB
                lg = [l + pltpu.roll(l, 64, 1) for l in st[i]]
                lg = [l + pltpu.roll(l, 32, 1) for l in lg]
                for w in range(W):
                    if masked and r0 < DIL * w:
                        pos = lax.broadcasted_iota(jnp.int32, (RB, 128), 0) + (b * TB + r0)
                        lg[w] = jnp.where(pos >= DIL * w, lg[w], NEG / SCALE)
                mx = jnp.maximum(jnp.maximum(jnp.maximum(lg[0], lg[1]), jnp.maximum(lg[2], lg[3])),
                                 jnp.maximum(jnp.maximum(lg[4], lg[5]), jnp.maximum(lg[6], lg[7])))
                e = [jnp.exp2((l - mx) * (SCALE * LOG2E)) for l in lg]
                den = ((e[0] + e[1]) + (e[2] + e[3])) + ((e[4] + e[5]) + (e[6] + e[7]))
                inv = pl.reciprocal(den, approx=True)
                st[i] = (e, inv * (2.0 - den * inv))
            def pv(i):
                r0 = i * RB
                e, inv = st.pop(i)
                for t in range(5):
                    acc = e[0] * rows(r0, VI[t], 0)
                    for w in range(1, W):
                        acc = acc + e[w] * rows(r0, VI[t], w)
                    if t == chain - 1:
                        buf[13, pl.ds(zs[0] + (HALO + TB), 8), :] = acc
                    o_v[2 * b + r0 // 128, r0 % 128:r0 % 128 + RB, t * 128:(t + 1) * 128] = (acc * inv).astype(bf16)
            def step(i):
                first = pf[i % len(pf)] == "1"
                if first and 0 <= i - lb < NA: pv(i - lb)
                if i < NA: logits(i)
                if 0 <= i - la < NA: softmax(i - la)
                if not first and 0 <= i - lb < NA: pv(i - lb)
            return [P(step, i) for i in range(NA + lb)]

        def token(buf, val):
            buf[13, pl.ds(zs[0] + (HALO + TB), 8), :] = val

        def paced(steps, chunks, buf):
            n, m = len(steps), len(chunks)
            if order == "pre":
                for t in chunks + steps: t()
                return
            if order == "post":
                for t in steps + chunks: t()
                return
            cuts = [0, g0] + [g0 + (n - g0 - glast) * (k + 1) // (m - 1) for k in range(m - 1)] + [n]
            for k in range(m + 1):
                for t in steps[cuts[k]:cuts[k + 1]]: t()
                if k < m:
                    v = chunks[k]()
                    if tok: token(buf, v)

        def proj_chunks(h, dst):
            def one(t0, t1):
                y = lax.dot_general(unpack(h[...]), unpack(wqkvT[t0 * 64:t1 * 64, :]), NT, preferred_element_type=f32)
                for t in range(t0, t1):
                    dst[t, HALO:HALO + TB, :] = y[:, (t - t0) * 128:(t - t0 + 1) * 128]
                return y[TB - 8:TB, (t1 - t0 - 1) * 128:(t1 - t0) * 128]
            return [P(one, t0, t1) for t0, t1 in grp]

        def wo(t0, nt=1):
            o = o_v[t0] if nt == 1 else jnp.concatenate([o_v[t] for t in range(t0, t0 + nt)], axis=0)
            a = lax.dot_general(unpack(woT[...]), o, NT, preferred_element_type=f32)
            for k in range(nt):
                aT[t0 + k] = a[:, k * 128:(k + 1) * 128]
            return a[D - 8:D, (nt - 1) * 128:nt * 128]

        def res(b, j):
            x1T[b, :, j:j + 128] = x_v[b, :, j:j + 128].astype(f32) + mod(2) * aT[2 * b + j // 128]

        def ln2(b, j):
            y = ln(x1T[b, :, j:j + 128]) * mod(4) + mod(3)
            for k0, kw in KT:
                h2[b, j // 2:j // 2 + 64, k0:k0 + kw] = pack(y[k0:k0 + kw, :].T)

        with scope("pro"):
            zs[0] = 0
            o_v[0] = jnp.zeros((128, 640), bf16)
            prep_qkv(0)
            copies["c"].wait()
            copies["x0"].wait()
            for j in range(3):
                mod_cols(j)
            ln1(0, hA)
        with scope("pro1"):
            proj(0, hA, A)
            prep_qkv(1)
            proj(1, hA, A)
            prep_qkv(2)
            proj(2, hA, A)
            for t in range(4, 14):
                A[t, 0:HALO, :] = jnp.broadcast_to(A[t, HALO:HALO + 1, :], (HALO, 128))
            copies["x1"].wait()
            ln1(1, hB)
            prep_wo()
            for b in range(2, NB):
                copies["x%d" % b].wait()

        def p1_body(j, _):
            with scope("p1it"):
                b = 2 * j
                ln1(b + 2, hA)
                paced(attn(b, A, True), [P(wo, jnp.maximum(b - 1, 0))] + proj_chunks(hB, B), A)
                halo(A, B)
                ln1(b + 3, hB)
                paced(attn(b + 1, B, False), [P(wo, b)] + proj_chunks(hA, A), B)
                halo(B, A)
        with scope("p1"):
            lax.fori_loop(0, NB // 2 - 1, p1_body, None)

        with scope("ep"):
            paced(attn(NB - 2, A, False), [P(wo, 5)] + proj_chunks(hB, B), A)
            halo(A, B)
            mod_cols(3)
            paced(attn(NB - 1, B, False), [P(wo, t) for t in range(6, 14)], B)
            wo(14, 2)
            for j in range(0, TB, 128):
                res(0, j)
                ln2(0, j)
            for n in ("wg", "wu", "wd"):
                copies[n].wait()

        def out_copy(i):
            s0 = i * TB if isinstance(i, int) else pl.multiple_of(i * TB, TB)
            return pltpu.make_async_copy(obuf.at[i], o_hbm.at[:, pl.ds(s0, TB)], osem.at[i])

        def ffn(i, _):
          with scope("ffnit"):
            nx = jnp.minimum(i + 1, NB - 1)
            side = [P(res, nx, 0), P(ln2, nx, 0), P(res, nx, 128), P(ln2, nx, 128)]
            todo = list(zip(fpos, side))
            def tick(step):
                while todo and todo[0][0] <= step:
                    todo.pop(0)[1]()
            h = unpack(h2[i])
            acc = None
            for j in range(NC):
                f0 = j * FC
                g = jnp.dot(h, wg_v[:, f0:f0 + FC], preferred_element_type=f32)
                tick(3 * j)
                u = jnp.dot(h, wu_v[:, f0:f0 + FC], preferred_element_type=f32)
                tick(3 * j + 1)
                y = lax.dot_general(wd_v[:, f0:f0 + FC], (g * u).astype(bf16), NT, preferred_element_type=f32)
                acc = y if acc is None else acc + y
                tick(3 * j + 2)
            tick(1 << 30)
            for j in range(0, TB, 128):
                obuf[i, :, j:j + 128] = (x1T[i, :, j:j + 128] + mod(5) * acc[:, j:j + 128]).astype(bf16)
            out_copy(i).start()
        with scope("ffn"):
            lax.fori_loop(0, NB, ffn, None)
        for i in range(NB):
            out_copy(i).wait()

    def fn(A_x, A_wqkv, A_wo, B_x, B_w_gate, B_w_up, B_w_down, c, w_mod):
        del B_x
        xT = A_x.reshape(S, D).T
        any_spec = pl.BlockSpec(memory_space=pl.ANY)
        V = pltpu.VMEM
        outT = pl.pallas_call(
            kernel,
            out_shape=jax.ShapeDtypeStruct((D, S), bf16),
            in_specs=[any_spec] * 8,
            out_specs=any_spec,
            scratch_shapes=[
                V((NB, D, TB), bf16), V((D, 3 * D), bf16), V((D, D), bf16),
                V((D, F), bf16), V((D, F), bf16), V((D, F), bf16),
                V((1, D), bf16), V((D, 6 * D), bf16),
                V((6 * D, 128), f32), V((5, 3 * D, 128), f32),
                V((14 * 64, D), u32), V((D // 2, 640), u32),
                V((TB // 2, D), u32), V((TB // 2, D), u32),
                V((14, HALO + TB + 8, 128), f32), V((14, HALO + TB + 8, 128), f32),
                V((S // 128, 128, 640), bf16), V((S // 128, D, 128), f32), V((NB, D, TB), f32), V((NB, TB // 2, D), u32),
                V((NB, D, TB), bf16),
                pltpu.SMEM((1,), jnp.int32),
                pltpu.SemaphoreType.DMA((24,)), pltpu.SemaphoreType.DMA((NB,)),
            ],
            compiler_params=pltpu.CompilerParams(vmem_limit_bytes=110 * 2**20, flags=flags),
            name=name,
        )(xT, A_wqkv, A_wo, B_w_gate, B_w_up, B_w_down.T, c, w_mod)
        return outT.T.reshape(1, S, D)
    fn.__name__ = name
    return fn


_fn = make()


@jax.jit
def pallas_adaLN_cond__sliding_local_dilated__glu_gated_bilinear__prompt_kernel(
        A_x, A_wqkv, A_wo, B_x, B_w_gate, B_w_up, B_w_down, c, w_mod):
    return _fn(A_x, A_wqkv, A_wo, B_x, B_w_gate, B_w_up, B_w_down, c, w_mod)
```

```python
import functools, contextlib
import jax, jax.numpy as jnp, numpy as np
from jax import lax
from jax.experimental import pallas as pl
from jax.experimental.pallas import tpu as pltpu

S, D, H, DH, W, DIL, F = 2048, 576, 32, 18, 8, 2, 4608
EPS = 1e-5
SCALE = DH ** -0.5
NEG = -1000000000.0
LOG2E = 1.4426950408889634
NT = (((1,), (1,)), ((), ()))
f32, bf16, u32 = jnp.float32, jnp.bfloat16, jnp.uint32
KT = [(k, min(128, D - k)) for k in range(0, D, 128)]
P = functools.partial
HALO = 16
RB = 8
QS = [[(0, 4 * t + j) for j in range(4)] for t in range(4)] + [[(0, 16), (0, 17), (2, 16), (2, 17)]]
KS = [[(1, 4 * t + j) for j in range(4)] for t in range(4)] + [[(1, 16), (1, 17), None, None]]
VS = [[(2, 4 * t + j) for j in range(4)] for t in range(4)]
TILES = QS[:4] + KS + VS + QS[4:]
QI, KI, VI = [0, 1, 2, 3, 13], [4, 5, 6, 7, 8], [9, 10, 11, 12, 13]
GROUPS = [(0, 4), (4, 9), (9, 14)]


def pack(x):
    return pltpu.bitcast(x.astype(bf16), u32)


def unpack(w):
    return pltpu.bitcast(w, bf16)


def make(TB=256, FC=1152, name="fused", scopes=False, fpos=(1, 2), lag=1, la=1, lb=2, chain=3, wo6=1, gt=2, g0=4, glast=2, tok=False, pf='0', grp=GROUPS, order='pre', flags=None, split=False, wog=2, pm=-1, pl2=4):
    NB = S // TB
    NC = F // FC
    NA = TB // RB
    scope = jax.named_scope if scopes else (lambda n: contextlib.nullcontext())

    def kernel(x_hbm, wqkv_hbm, wo_hbm, wg_hbm, wu_hbm, wd_hbm, c_hbm, wmod_hbm, o_hbm,
               x_v, wqkv_v, wo_v, wg_v, wu_v, wd_v, c_v, wmod_v,
               gate, rowv, tmp, wqkvT, woT, hA, hB, A0, A1, B0, B1, o_v, aT, obuf, zs, sems, osem):
        A, B = (A0, A1), (B0, B1)
        def tile(buf, t):
            return buf[1].at[t - 9] if (split and 9 <= t < 13) else buf[0].at[t]
        names = []
        copies = {}
        def add(name, src, dst):
            copies[name] = pltpu.make_async_copy(src, dst, sems.at[len(names)])
            names.append(name)
        def cols(name, src, dst, lo, hi):
            add(name, src.at[:, lo:hi], dst.at[:, lo:hi])
        QKV_CUT = [0, 640, 1152, 3 * D]
        MOD_CUT = [0, 384, 768, 1152, 6 * D]
        add("c", c_hbm, c_v)
        cols("wqkv0", wqkv_hbm, wqkv_v, QKV_CUT[0], QKV_CUT[1])
        add("x0", x_hbm.at[:, 0:TB], x_v.at[0])
        for j in range(3):
            cols("wmod%d" % j, wmod_hbm, wmod_v, MOD_CUT[j], MOD_CUT[j + 1])
        for p in (1, 2):
            cols("wqkv%d" % p, wqkv_hbm, wqkv_v, QKV_CUT[p], QKV_CUT[p + 1])
        add("x1", x_hbm.at[:, TB:2 * TB], x_v.at[1])
        add("wo", wo_hbm, wo_v)
        for b in range(2, NB):
            add("x%d" % b, x_hbm.at[:, b * TB:(b + 1) * TB], x_v.at[b])
        cols("wmod3", wmod_hbm, wmod_v, MOD_CUT[3], MOD_CUT[4])
        add("wg", wg_hbm, wg_v)
        add("wu", wu_hbm, wu_v)
        add("wd", wd_hbm, wd_v)
        for n in names:
            copies[n].start()

        def prep_qkv(p):
            for t, (k0, kw) in enumerate(KT):
                for n0 in range(QKV_CUT[p], QKV_CUT[p + 1], 128):
                    nw = min(128, 3 * D - n0)
                    blk = wqkv_v[k0:k0 + kw, n0:n0 + nw].astype(f32)
                    tmp[t, n0:n0 + nw, 0:kw] = blk.T
            for t, (k0, kw) in enumerate(KT):
                for ti in range(*GROUPS[p]):
                    for j, slot in enumerate(TILES[ti]):
                        r0 = (ti * 128 + j * H) // 2
                        if slot is None:
                            wqkvT[r0:r0 + H // 2, k0:k0 + kw] = jnp.zeros((H // 2, kw), u32)
                        else:
                            rows = tmp[t, pl.ds(slot[0] * D + slot[1], H, stride=DH), :]
                            wqkvT.bitcast(bf16)[2 * r0:2 * r0 + H, k0:k0 + kw] = rows[:, 0:kw].astype(bf16)

        def prep_wo():
            for t, (n0, nw) in enumerate(KT):
                tmp[t, 0:D, 0:nw] = wo_v[:, n0:n0 + nw].astype(f32)
            for t, (n0, nw) in enumerate(KT):
                for ti in range(5):
                    ds = [4 * ti + j for j in range(4)] if ti < 4 else [None, None, 16, 17]
                    parts = [jnp.zeros((H, nw), f32) if d is None else tmp[t, pl.ds(d, H, stride=DH), :][:, 0:nw] for d in ds]
                    woT[n0 // 2:(n0 + nw) // 2, ti * 128:(ti + 1) * 128] = pack(jnp.concatenate(parts, axis=0).T)

        def silu_c():
            cf = c_v[...].astype(f32)
            return (cf * jax.nn.sigmoid(cf)).astype(bf16)

        def mod_a():
            sc = jnp.broadcast_to(silu_c(), (16, D))
            parts = []
            for j in range(3):
                copies["wmod%d" % j].wait()
                parts.append(jnp.dot(sc, wmod_v[:, MOD_CUT[j]:MOD_CUT[j + 1]], preferred_element_type=f32)[0:8, :])
            m = jnp.concatenate(parts, axis=1)
            rowv[0, :, 0:D] = m[:, 0:D]
            rowv[1, :, 0:D] = 1.0 + m[:, D:2 * D]

        def mod_b():
            sc = jnp.broadcast_to(silu_c(), (16, D))
            m = jnp.dot(sc, wmod_v[:, 2 * D:6 * D], preferred_element_type=f32)[0:8, :]
            rowv[2, :, 0:D] = m[:, D:2 * D]
            rowv[3, :, 0:D] = 1.0 + m[:, 2 * D:3 * D]
            for i, g in enumerate((m[:, 0:D], m[:, 3 * D:4 * D])):
                for k0, kw in KT:
                    gate[i, k0:k0 + kw, :] = jnp.broadcast_to(g[0:1, k0:k0 + kw], (128, kw)).T

        def ln_to_rows(xf, h, j, i_shift, i_scale):
            m = jnp.sum(xf, axis=0, keepdims=True) * (1.0 / D)
            d = xf - m
            v = jnp.sum(d * d, axis=0, keepdims=True) * (1.0 / D)
            n = d * lax.rsqrt(v + EPS)
            for k0, kw in KT:
                y = n[k0:k0 + kw, :].T * rowv[i_scale, 0:1, k0:k0 + kw] + rowv[i_shift, 0:1, k0:k0 + kw]
                h[j:j + 128, k0:k0 + kw] = y.astype(bf16)

        def ln1(b, h):
            for j in range(0, TB, 128):
                ln_to_rows(x_v[b, :, j:j + 128].astype(f32), h.bitcast(bf16), j, 0, 1)

        def proj(p, h, dst):
            t0, t1 = GROUPS[p]
            y = lax.dot_general(h.bitcast(bf16)[...], wqkvT.bitcast(bf16)[t0 * 128:t1 * 128, :], NT, preferred_element_type=f32)
            for t in range(t0, t1):
                tile(dst, t)[HALO:HALO + TB, :] = y[:, (t - t0) * 128:(t - t0 + 1) * 128]

        def halo(src, dst):
            for t in range(4, 14):
                tile(dst, t)[0:HALO, :] = tile(src, t)[TB:TB + HALO, :]

        def attn(b, buf, masked):
            st = {}
            def rows(r0, t, w):
                r = HALO + r0 - DIL * w
                return tile(buf, t)[r:r + RB, :]
            def logits(i):
                r0 = i * RB
                q = [rows(r0, t, 0) for t in QI]
                st[i] = []
                for w in range(W):
                    acc = q[0] * rows(r0, KI[0], w)
                    for t in range(1, 5):
                        acc = acc + q[t] * rows(r0, KI[t], w)
                    st[i].append(acc)
            def softmax(i):
                r0 = i * RB
                lg = [l + pltpu.roll(l, 64, 1) for l in st[i]]
                lg = [l + pltpu.roll(l, 32, 1) for l in lg]
                for w in range(W):
                    if masked and r0 < DIL * w:
                        pos = lax.broadcasted_iota(jnp.int32, (RB, 128), 0) + (b * TB + r0)
                        lg[w] = jnp.where(pos >= DIL * w, lg[w], NEG / SCALE)
                mx = jnp.maximum(jnp.maximum(jnp.maximum(lg[0], lg[1]), jnp.maximum(lg[2], lg[3])),
                                 jnp.maximum(jnp.maximum(lg[4], lg[5]), jnp.maximum(lg[6], lg[7])))
                e = [jnp.exp2((l - mx) * (SCALE * LOG2E)) for l in lg]
                den = ((e[0] + e[1]) + (e[2] + e[3])) + ((e[4] + e[5]) + (e[6] + e[7]))
                inv = pl.reciprocal(den, approx=True)
                st[i] = (e, inv * (2.0 - den * inv))
            def pv(i):
                r0 = i * RB
                e, inv = st.pop(i)
                for t in range(5):
                    acc = e[0] * rows(r0, VI[t], 0)
                    for w in range(1, W):
                        acc = acc + e[w] * rows(r0, VI[t], w)
                    if t == chain - 1:
                        buf[0][13, pl.ds(zs[0] + (HALO + TB), 8), :] = acc
                    o_v[2 * b + r0 // 128, r0 % 128:r0 % 128 + RB, t * 128:(t + 1) * 128] = (acc * inv).astype(bf16)
            def step(i):
                first = pf[i % len(pf)] == "1"
                if first and 0 <= i - lb < NA: pv(i - lb)
                if i < NA: logits(i)
                if 0 <= i - la < NA: softmax(i - la)
                if not first and 0 <= i - lb < NA: pv(i - lb)
            return [P(step, i) for i in range(NA + lb)]

        def token(buf, val):
            buf[0][13, pl.ds(zs[0] + (HALO + TB), 8), :] = val

        def paced(steps, chunks, buf):
            n, m = len(steps), len(chunks)
            if order == "pre":
                for t in chunks + steps: t()
                return
            if order == "post":
                for t in steps + chunks: t()
                return
            cuts = [0, g0] + [g0 + (n - g0 - glast) * (k + 1) // (m - 1) for k in range(m - 1)] + [n]
            for k in range(m + 1):
                for t in steps[cuts[k]:cuts[k + 1]]: t()
                if k < m:
                    v = chunks[k]()
                    if tok: token(buf, v)

        def proj_chunks(h, dst):
            def one(t0, t1):
                y = lax.dot_general(h.bitcast(bf16)[...], wqkvT.bitcast(bf16)[t0 * 128:t1 * 128, :], NT, preferred_element_type=f32)
                for t in range(t0, t1):
                    tile(dst, t)[HALO:HALO + TB, :] = y[:, (t - t0) * 128:(t - t0 + 1) * 128]
                return y[TB - 8:TB, (t1 - t0 - 1) * 128:(t1 - t0) * 128]
            return [P(one, t0, t1) for t0, t1 in grp]

        def wo(t0, nt=1):
            o = o_v[t0] if nt == 1 else jnp.concatenate([o_v[t] for t in range(t0, t0 + nt)], axis=0)
            a = lax.dot_general(woT.bitcast(bf16)[0:D, :], o, NT, preferred_element_type=f32)
            for k in range(nt):
                aT[t0 + k] = a[:, k * 128:(k + 1) * 128]
            return a[D - 8:D, (nt - 1) * 128:nt * 128]

        def x1(b, j):
            return x_v[b, :, j:j + 128].astype(f32) + gate[0] * aT[2 * b + j // 128]

        def h2(slot):
            return woT.bitcast(bf16).at[pl.ds(pl.multiple_of(D + slot * TB, 16), TB)]

        def ln2(b, j, slot):
            ln_to_rows(x1(b, j), h2(slot), j, 2, 3)

        with scope("pro"):
            zs[0] = 0
            copies["c"].wait()
            copies["wqkv0"].wait()
            prep_qkv(0)
            copies["x0"].wait()
            mod_a()
            ln1(0, hA)
        with scope("pro1"):
            copies["wqkv1"].wait()
            proj(0, hA, A)
            prep_qkv(1)
            copies["wqkv2"].wait()
            proj(1, hA, A)
            prep_qkv(2)
            copies["x1"].wait()
            copies["wo"].wait()
            proj(2, hA, A)
            ln1(1, hB)
            prep_wo()
            for t in range(4, 14):
                tile(A, t)[0:HALO, :] = jnp.broadcast_to(tile(A, t)[HALO:HALO + 1, :], (HALO, 128))
            copies["x2"].wait()

        with scope("st0"):
            ln1(2, hA)
            paced(attn(0, A, True), proj_chunks(hB, B), A)
            halo(A, B)
            for b in range(3, NB):
                copies["x%d" % b].wait()

        def p1_body(j, _):
            with scope("p1it"):
                b = 2 * j + 1
                ln1(b + 2, hB)
                paced(attn(b, B, False), [P(wo, b - 1)] + proj_chunks(hA, A), B)
                halo(B, A)
                ln1(jnp.minimum(b + 3, NB - 1), hA)
                paced(attn(b + 1, A, False), [P(wo, b)] + proj_chunks(hB, B), A)
                halo(A, B)
        with scope("p1"):
            lax.fori_loop(0, NB // 2 - 1, p1_body, None)

        with scope("ep"):
            copies["wmod3"].wait()
            if pm < 0: mod_b()
            for k, t in enumerate(range(6, 14, 2)):
                if k == pm: mod_b()
                if k == pl2:
                    for j in range(0, TB, 128):
                        ln2(0, j, zs[0])
                wo(t, 2)
            for t in attn(NB - 1, B, False): t()
            wo(14, 2)
            if pl2 > 3:
                for j in range(0, TB, 128):
                    ln2(0, j, 0)
            for n in ("wg", "wu", "wd"):
                copies[n].wait()

        def out_copy(i):
            s0 = i * TB if isinstance(i, int) else pl.multiple_of(i * TB, TB)
            return pltpu.make_async_copy(obuf.at[i], o_hbm.at[:, pl.ds(s0, TB)], osem.at[i])

        def ffn(i, _):
          with scope("ffnit"):
            nx = jnp.minimum(i + 1, NB - 1)
            cur = i % 2
            side = [P(ln2, nx, j, 1 - cur) for j in range(0, TB, 128)]
            todo = list(zip(fpos, side))
            def tick(step):
                while todo and todo[0][0] <= step:
                    todo.pop(0)[1]()
            acc = None
            hh = {}
            for j in range(NC + lag):
                if j < NC:
                    f0 = j * FC
                    h = h2(cur)[:, 0:D]
                    g = jnp.dot(h, wg_v[:, f0:f0 + FC], preferred_element_type=f32)
                    u = jnp.dot(h, wu_v[:, f0:f0 + FC], preferred_element_type=f32)
                    hh[j] = (g * u).astype(bf16)
                tick(j)
                if j >= lag:
                    f0 = (j - lag) * FC
                    y = lax.dot_general(wd_v[:, f0:f0 + FC], hh.pop(j - lag), NT, preferred_element_type=f32)
                    acc = y if acc is None else acc + y
            tick(1 << 30)
            for j in range(0, TB, 128):
                obuf[i, :, j:j + 128] = (x1(i, j) + gate[1] * acc[:, j:j + 128]).astype(bf16)
            out_copy(i).start()
        with scope("ffn"):
            lax.fori_loop(0, NB, ffn, None)
        for i in range(NB):
            out_copy(i).wait()

    def fn(A_x, A_wqkv, A_wo, B_x, B_w_gate, B_w_up, B_w_down, c, w_mod):
        del B_x
        xT = A_x.reshape(S, D).T
        any_spec = pl.BlockSpec(memory_space=pl.ANY)
        V = pltpu.VMEM
        outT = pl.pallas_call(
            kernel,
            out_shape=jax.ShapeDtypeStruct((D, S), bf16),
            in_specs=[any_spec] * 8,
            out_specs=any_spec,
            scratch_shapes=[
                V((NB, D, TB), bf16), V((D, 3 * D), bf16), V((D, D), bf16),
                V((D, F), bf16), V((D, F), bf16), V((D, F), bf16),
                V((1, D), bf16), V((D, 6 * D), bf16),
                V((2, D, 128), f32), V((4, 8, 640), f32), V((5, 3 * D, 128), f32),
                V((14 * 64, D), u32), V((D // 2 + TB + 8, 640), u32),
                V((TB // 2, D), u32), V((TB // 2, D), u32),
                V((14, HALO + TB + 8, 128), f32), V((4, HALO + TB, 128), f32), V((14, HALO + TB + 8, 128), f32), V((4, HALO + TB, 128), f32),
                V((S // 128, 128, 640), bf16), V((S // 128, D, 128), f32), V((NB, D, TB), bf16),
                pltpu.SMEM((1,), jnp.int32),
                pltpu.SemaphoreType.DMA((24,)), pltpu.SemaphoreType.DMA((NB,)),
            ],
            compiler_params=pltpu.CompilerParams(vmem_limit_bytes=110 * 2**20, flags=flags),
            name=name,
        )(xT, A_wqkv, A_wo, B_w_gate, B_w_up, B_w_down.T, c, w_mod)
        return outT.T.reshape(1, S, D)
    fn.__name__ = name
    return fn


_fn = make()


@jax.jit
def pallas_adaLN_cond__sliding_local_dilated__glu_gated_bilinear__prompt_kernel(
        A_x, A_wqkv, A_wo, B_x, B_w_gate, B_w_up, B_w_down, c, w_mod):
    return _fn(A_x, A_wqkv, A_wo, B_x, B_w_gate, B_w_up, B_w_down, c, w_mod)
```

```python
import functools, contextlib
import jax, jax.numpy as jnp, numpy as np
from jax import lax
from jax.experimental import pallas as pl
from jax.experimental.pallas import tpu as pltpu

S, D, H, DH, W, DIL, F = 2048, 576, 32, 18, 8, 2, 4608
EPS = 1e-5
SCALE = DH ** -0.5
NEG = -1000000000.0
LOG2E = 1.4426950408889634
NT = (((1,), (1,)), ((), ()))
f32, bf16, u32 = jnp.float32, jnp.bfloat16, jnp.uint32
KT = [(k, min(128, D - k)) for k in range(0, D, 128)]
P = functools.partial
HALO = 16
RB = 8
TB = 256
NB = S // TB


def make(FC=1152, name="fused", scopes=False, fpos=(1, 2), lag=1, la=2, lb=2, chain=4, pf="0", grp=((4, 12), (0, 4)),
         flags=None, pm=-1, only=None, ypos=0, lnpos=2, wopos=0, vord="t", epc=None, s0c=None, lt=1, vt=0, split=True, lend=False, lnk=(1, 3)):
    NC = F // FC
    scope = jax.named_scope if scopes else (lambda n: contextlib.nullcontext())

    def kernel(x_hbm, wqkv_hbm, wo_hbm, wg_hbm, wu_hbm, wd_hbm, c_hbm, wmod_hbm, o_hbm,
               x_v, wqkv_v, wo_v, wg_v, wu_v, wd_v, c_v, wmod_v,
               gate, rowv, tmp, wqkvT, woT, hA, hB, A0, A1, B0, B1, o_v, aT, obuf, zs, sems, osem):
        class Buf:
            def __init__(self, qk, v):
                self.qk, self.v = qk, (v if split else qk)
            def __getitem__(self, idx):
                return (self.v if idx[0] in (8, 9, 10, 11, 14) else self.qk)[idx]
            def __setitem__(self, idx, val):
                (self.v if idx[0] in (8, 9, 10, 11, 14) else self.qk)[idx] = val
        A, B = Buf(A0, A1), Buf(B0, B1)
        names = []
        copies = {}
        def add(name, src, dst):
            copies[name] = pltpu.make_async_copy(src, dst, sems.at[len(names)])
            names.append(name)
        def cols(name, src, dst, lo, hi):
            add(name, src.at[:, lo:hi], dst.at[:, lo:hi])
        QKV_CUT = [0, 640, 1152, 3 * D]
        MOD_CUT = [0, 384, 768, 1152, 6 * D]
        if not only:
            add("c", c_hbm, c_v)
            cols("wqkv0", wqkv_hbm, wqkv_v, QKV_CUT[0], QKV_CUT[1])
            add("x0", x_hbm.at[:, 0:TB], x_v.at[0])
            for j in range(3):
                cols("wmod%d" % j, wmod_hbm, wmod_v, MOD_CUT[j], MOD_CUT[j + 1])
            for p in (1, 2):
                cols("wqkv%d" % p, wqkv_hbm, wqkv_v, QKV_CUT[p], QKV_CUT[p + 1])
            add("x1", x_hbm.at[:, TB:2 * TB], x_v.at[1])
            add("wo", wo_hbm, wo_v)
            for b in range(2, NB):
                add("x%d" % b, x_hbm.at[:, b * TB:(b + 1) * TB], x_v.at[b])
            cols("wmod3", wmod_hbm, wmod_v, MOD_CUT[3], MOD_CUT[4])
            add("wg", wg_hbm, wg_v)
            add("wu", wu_hbm, wu_v)
            add("wd", wd_hbm, wd_v)
        for n in names:
            copies[n].start()
        def wait(*ns):
            if not only:
                for n in ns: copies[n].wait()

        def prep_qkv(p):
            for t, (k0, kw) in enumerate(KT):
                for n0 in range(QKV_CUT[p], QKV_CUT[p + 1], 128):
                    nw = min(128, 3 * D - n0)
                    tmp[t, n0:n0 + nw, 0:kw] = wqkv_v[k0:k0 + kw, n0:n0 + nw].astype(f32).T
            for t, (k0, kw) in enumerate(KT):
                for d in range(DH):
                    r0 = (p * 16 + d) * H if d < 16 else (48 + 2 * p + d - 16) * H
                    rows = tmp[t, pl.ds(p * D + d, H, stride=DH), :]
                    wqkvT.bitcast(bf16)[r0:r0 + H, k0:k0 + kw] = rows[:, 0:kw].astype(bf16)

        def prep_wo():
            for t, (n0, nw) in enumerate(KT):
                tmp[t, 0:D, 0:nw] = wo_v[:, n0:n0 + nw].astype(f32)
            for t, (n0, nw) in enumerate(KT):
                for ti in range(6):
                    ds = [4 * ti + j for j in range(4)] if ti < 4 else ([16, 17, None, None], [None, None, 16, 17])[ti - 4]
                    parts = [jnp.zeros((H, nw), f32) if d is None else tmp[t, pl.ds(d, H, stride=DH), :][:, 0:nw] for d in ds]
                    y = jnp.concatenate(parts, axis=0).T.astype(bf16)
                    c0 = (ti + 1) * 128 if ti < 4 else (0, 640)[ti - 4]
                    woT.bitcast(bf16)[n0:n0 + nw, c0:c0 + 128] = y

        def silu_c():
            cf = c_v[...].astype(f32)
            return jnp.broadcast_to((cf * jax.nn.sigmoid(cf)).astype(bf16), (16, D))

        def mod_a():
            sc = silu_c()
            parts = []
            for j in range(3):
                wait("wmod%d" % j)
                parts.append(jnp.dot(sc, wmod_v[:, MOD_CUT[j]:MOD_CUT[j + 1]], preferred_element_type=f32)[0:8, :])
            m = jnp.concatenate(parts, axis=1)
            rowv[0, :, 0:D] = m[:, 0:D]
            rowv[1, :, 0:D] = 1.0 + m[:, D:2 * D]

        def mod_b():
            m = jnp.dot(silu_c(), wmod_v[:, 2 * D:6 * D], preferred_element_type=f32)[0:8, :]
            rowv[2, :, 0:D] = m[:, D:2 * D]
            rowv[3, :, 0:D] = 1.0 + m[:, 2 * D:3 * D]
            for i, g in enumerate((m[:, 0:D], m[:, 3 * D:4 * D])):
                for k0, kw in KT:
                    gate[i, k0:k0 + kw, :] = jnp.broadcast_to(g[0:1, k0:k0 + kw], (128, kw)).T

        def ln_to_rows(xf, h, j, i_shift, i_scale):
            m = jnp.sum(xf, axis=0, keepdims=True) * (1.0 / D)
            d = xf - m
            v = jnp.sum(d * d, axis=0, keepdims=True) * (1.0 / D)
            n = d * lax.rsqrt(v + EPS)
            for k0, kw in KT:
                y = n[k0:k0 + kw, :].T * rowv[i_scale, 0:1, k0:k0 + kw] + rowv[i_shift, 0:1, k0:k0 + kw]
                h[j:j + 128, k0:k0 + kw] = y.astype(bf16)
                if k0 == 384: last = y[120:128, :]
            return last

        def ln1(b, h):
            for j in range(0, TB, 128):
                ln_to_rows(x_v[b, :, j:j + 128].astype(f32), h.bitcast(bf16), j, 0, 1)

        def proj(t0, t1, h, dst):
            y = lax.dot_general(h.bitcast(bf16)[:, 0:D], wqkvT.bitcast(bf16)[t0 * 128:t1 * 128, 0:D], NT, preferred_element_type=f32)
            for t in range(t0, t1):
                dst[t, HALO:HALO + TB, :] = y[:, (t - t0) * 128:(t - t0 + 1) * 128]

        def proj_rest(h, dst):
            y = lax.dot_general(wqkvT.bitcast(bf16)[12 * 128:3 * D, 0:D], h.bitcast(bf16)[:, 0:D], NT, preferred_element_type=f32)
            for p in range(3):
                yp = y[64 * p:64 * p + 64, :]
                dst[12 + p, HALO:HALO + 128, :] = jnp.concatenate([yp[:, 0:128], yp[:, 128:256]], axis=0).T

        def low_half(rows):
            return lax.broadcasted_iota(jnp.int32, (rows, 128), 1) < 64

        def halo(src, dst):
            for t in range(4, 12):
                dst[t, 0:HALO, :] = src[t, TB:TB + HALO, :]
            for t in (13, 14):
                both = jnp.where(low_half(HALO), dst[t, 128:128 + HALO, :], src[t, 128:128 + HALO, :])
                dst[t, 0:HALO, :] = pltpu.roll(both, 64, 1)

        def halo_first(dst):
            for t in range(4, 12):
                dst[t, 0:HALO, :] = jnp.broadcast_to(dst[t, HALO:HALO + 1, :], (HALO, 128))
            for t in (13, 14):
                first = jnp.broadcast_to(dst[t, HALO:HALO + 1, :], (HALO, 128))
                dst[t, 0:HALO, :] = jnp.where(low_half(HALO), first, pltpu.roll(dst[t, 128:128 + HALO, :], 64, 1))

        def attn(b, buf, masked=False, lb=lb, la=la, chain=chain, pf=pf, vord=vord, lt=lt, vt=vt, side=()):
            st = {}
            NP = 128 // RB
            lane = lax.broadcasted_iota(jnp.int32, (RB, 128), 1)
            lo = lane < 64
            even = (lane & 32) == 0
            def rows(r0, t, w):
                r = HALO + r0 - DIL * w
                return buf[t, r:r + RB, :]
            def logits(i):
                r0 = i * RB
                q = [[rows(r0 + o, t, 0) for t in range(4)] for o in (0, 128)]
                qr = rows(r0, 12, 0)
                out = []
                for w in range(W):
                    p = []
                    for k, o in enumerate((0, 128)):
                        acc = q[k][0] * rows(r0 + o, 4, w)
                        for t in range(1, 4):
                            acc = acc + q[k][t] * rows(r0 + o, 4 + t, w)
                        p.append(acc)
                    out.append((jnp.where(lo, p[0], p[1]) + qr * rows(r0, 13, w), jnp.where(lo, p[1], p[0])))
                    if lt and w % lt == lt - 1 and (lend or w < W - 1):
                        buf[0, pl.ds(zs[0] + (HALO + TB), 8), :] = p[1]
                st[i] = out
            def softmax(i):
                r0 = i * RB
                lg = [a + pltpu.roll(c, 64, 1) for a, c in st[i]]
                lg = [l + jnp.where(even, pltpu.roll(l, 96, 1), pltpu.roll(l, 32, 1)) for l in lg]
                for w in range(W):
                    if masked and r0 < DIL * w:
                        pos = lax.broadcasted_iota(jnp.int32, (RB, 128), 0) + r0
                        lg[w] = jnp.where(lo & (pos < DIL * w), NEG / SCALE, lg[w])
                mx = jnp.maximum(jnp.maximum(jnp.maximum(lg[0], lg[1]), jnp.maximum(lg[2], lg[3])),
                                 jnp.maximum(jnp.maximum(lg[4], lg[5]), jnp.maximum(lg[6], lg[7])))
                e = [jnp.exp2((l - mx) * (SCALE * LOG2E)) for l in lg]
                den = ((e[0] + e[1]) + (e[2] + e[3])) + ((e[4] + e[5]) + (e[6] + e[7]))
                inv = pl.reciprocal(den, approx=True)
                inv = inv * (2.0 - den * inv)
                st[i] = [x * inv for x in e]
            def pv(i):
                r0 = i * RB
                p = st.pop(i)
                pp = []
                for x in p:
                    r = pltpu.roll(x, 64, 1)
                    pp.append((jnp.where(lo, x, r), jnp.where(lo, r, x)))
                outs = [(o, t) for t in range(4) for o in (0, 1)] + [None]
                acc = {}
                order = [(k, w) for k in outs for w in range(W)] if vord == "t" else [(k, w) for w in range(W) for k in outs]
                for k, w in order:
                    pr = p[w] * rows(r0, 14, w) if k is None else pp[w][k[0]] * rows(r0 + 128 * k[0], 8 + k[1], w)
                    acc[k] = pr if w == 0 else acc[k] + pr
                    if vt and vord == "w" and k is None and w % vt == vt - 1 and w < W - 1:
                        buf[8, pl.ds(zs[0] + (HALO + TB), 8), :] = pr
                    if w == W - 1:
                        if vt and vord == "t" and outs.index(k) % vt == vt - 1:
                            buf[8, pl.ds(zs[0] + (HALO + TB), 8), :] = acc[k]
                        if k == outs[chain - 1]:
                            buf[0, pl.ds(zs[0] + (HALO + TB), 8), :] = acc[k]
                        y = acc[k].astype(bf16)
                        if k is None:
                            o_v[2 * b, r0:r0 + RB, 0:128] = y
                            o_v[2 * b + 1, r0:r0 + RB, 512:640] = y
                        else:
                            c0 = (k[1] + 1 - k[0]) * 128
                            o_v[2 * b + k[0], r0:r0 + RB, c0:c0 + 128] = y
            for i in range(NP + lb):
                for k, t in side:
                    if k == i: buf[0, pl.ds(zs[0] + (HALO + TB), 8), :] = t()
                first = pf[i % len(pf)] == "1"
                if first and 0 <= i - lb < NP: pv(i - lb)
                if i < NP: logits(i)
                if 0 <= i - la < NP: softmax(i - la)
                if not first and 0 <= i - lb < NP: pv(i - lb)

        def wo(t, odd):
            c0 = 128 * odd
            aT[t] = lax.dot_general(woT.bitcast(bf16)[0:D, c0:c0 + 640], o_v[t], NT, preferred_element_type=f32)

        def x1(b, j):
            return x_v[b, :, j:j + 128].astype(f32) + gate[0] * aT[2 * b + j // 128]

        def h2(slot):
            r0 = D + slot * TB
            return woT.bitcast(bf16).at[pl.ds(r0 if isinstance(r0, int) else pl.multiple_of(r0, 16), TB)]

        def ln2(b, j, slot):
            ln_to_rows(x1(b, j), h2(slot), j, 2, 3)

        if not only:
            with scope("pro"):
                zs[0] = 0
                wait("c", "wqkv0")
                prep_qkv(0)
                wait("x0")
                mod_a()
                ln1(0, hA)
            with scope("pro1"):
                wait("wqkv1")
                proj(0, 4, hA, A)
                prep_qkv(1)
                wait("wqkv2")
                proj(4, 8, hA, A)
                prep_qkv(2)
                wait("x1", "wo")
                proj_rest(hA, A)
                proj(8, 12, hA, A)
                ln1(1, hB)
                prep_wo()
                halo_first(A)
                wait("x2")

        def stage(b, cur, nxt, h_cur, h_nxt, odd=None, **kw):
            b2 = b + 2 if isinstance(b, int) else jnp.minimum(b + 2, NB - 1)
            ts = [P(proj, t0, t1, h_cur, nxt) for t0, t1 in grp]
            ts = ts[:ypos] + [P(proj_rest, h_cur, nxt)] + ts[ypos:]
            if odd is not None:
                ts = ts[:wopos] + [P(wo, b - 1, odd)] + ts[wopos:]
            if lnpos == 0: ln1(b2, h_nxt)
            for t in ts: t()
            if lnpos == 1: ln1(b2, h_nxt)
            side = ()
            if lnpos == 2:
                side = list(zip(lnk, [P(lambda j: ln_to_rows(x_v[b2, :, j:j + 128].astype(f32), h_nxt.bitcast(bf16), j, 0, 1), j) for j in (0, 128)]))
            attn(b, cur, side=side, **kw)
            halo(cur, nxt)

        if only in (None, "st0"):
            with scope("st0"):
                stage(0, A, B, hA, hB, masked=True, **(s0c or {})) if False else stage(0, A, B, hB, hA, masked=True, **(s0c or {}))
                wait(*["x%d" % b for b in range(3, NB)])

        def p1_body(j, _):
            with scope("p1it"):
                b = 2 * j + 1
                stage(b, B, A, hA, hB, 0)
                stage(b + 1, A, B, hB, hA, 1)
        if only in (None, "p1"):
            with scope("p1"):
                lax.fori_loop(0, NB // 2 - 1, p1_body, None)

        if only in (None, "ep"):
            with scope("ep"):
                wait("wmod3")
                if pm < 0: mod_b()
                for t in range(6, 14):
                    if t == pm: mod_b()
                    wo(t, t % 2)
                attn(NB - 1, B, **(epc or {}))
                wo(14, 0)
                wo(15, 1)
                for j in range(0, TB, 128):
                    ln2(0, j, 0)
                wait("wg", "wu", "wd")
        if only: return

        def out_copy(i):
            s0 = i * TB if isinstance(i, int) else pl.multiple_of(i * TB, TB)
            return pltpu.make_async_copy(obuf.at[i], o_hbm.at[:, pl.ds(s0, TB)], osem.at[i])

        def ffn(i, _):
          with scope("ffnit"):
            nx = jnp.minimum(i + 1, NB - 1)
            cur = i % 2
            todo = list(zip(fpos, [P(ln2, nx, j, 1 - cur) for j in range(0, TB, 128)]))
            def tick(step):
                while todo and todo[0][0] <= step:
                    todo.pop(0)[1]()
            acc = None
            hh = {}
            for j in range(NC + lag):
                if j < NC:
                    f0 = j * FC
                    h = h2(cur)[:, 0:D]
                    g = jnp.dot(h, wg_v[:, f0:f0 + FC], preferred_element_type=f32)
                    u = jnp.dot(h, wu_v[:, f0:f0 + FC], preferred_element_type=f32)
                    hh[j] = (g * u).astype(bf16)
                tick(j)
                if j >= lag:
                    f0 = (j - lag) * FC
                    y = lax.dot_general(wd_v[:, f0:f0 + FC], hh.pop(j - lag), NT, preferred_element_type=f32)
                    acc = y if acc is None else acc + y
            tick(1 << 30)
            for j in range(0, TB, 128):
                obuf[i, :, j:j + 128] = (x1(i, j) + gate[1] * acc[:, j:j + 128]).astype(bf16)
            out_copy(i).start()
        with scope("ffn"):
            lax.fori_loop(0, NB, ffn, None)
        for i in range(NB):
            out_copy(i).wait()

    def fn(A_x, A_wqkv, A_wo, B_x, B_w_gate, B_w_up, B_w_down, c, w_mod):
        del B_x
        xT = A_x.reshape(S, D).T
        any_spec = pl.BlockSpec(memory_space=pl.ANY)
        V = pltpu.VMEM
        outT = pl.pallas_call(
            kernel,
            out_shape=jax.ShapeDtypeStruct((D, S), bf16),
            in_specs=[any_spec] * 8,
            out_specs=any_spec,
            scratch_shapes=[
                V((NB, D, TB), bf16), V((D, 3 * D), bf16), V((D, D), bf16),
                V((D, F), bf16), V((D, F), bf16), V((D, F), bf16),
                V((1, D), bf16), V((D, 6 * D), bf16),
                V((2, D, 128), f32), V((4, 8, 640), f32), V((5, 3 * D, 128), f32),
                V((3 * D // 2, 640), u32), V((D // 2 + TB, 768), u32),
                V((TB // 2, 640), u32), V((TB // 2, 640), u32),
                *[V((15, HALO + TB + 8, 128), f32)] * 4,
                V((S // 128, 128, 640), bf16), V((S // 128, D, 128), f32),
                V((NB, D, TB), bf16),
                pltpu.SMEM((1,), jnp.int32),
                pltpu.SemaphoreType.DMA((24,)), pltpu.SemaphoreType.DMA((NB,)),
            ],
            compiler_params=pltpu.CompilerParams(vmem_limit_bytes=110 * 2**20, flags=flags),
            name=name,
        )(xT, A_wqkv, A_wo, B_w_gate, B_w_up, B_w_down.T, c, w_mod)
        return outT.T.reshape(1, S, D)
    fn.__name__ = name
    return fn


_fn = make()


@jax.jit
def pallas_adaLN_cond__sliding_local_dilated__glu_gated_bilinear__prompt_kernel(
        A_x, A_wqkv, A_wo, B_x, B_w_gate, B_w_up, B_w_down, c, w_mod):
    return _fn(A_x, A_wqkv, A_wo, B_x, B_w_gate, B_w_up, B_w_down, c, w_mod)
```

```python
import jax
import jax.numpy as jnp
from jax import lax
from jax.experimental import pallas as pl
from jax.experimental.pallas import tpu as pltpu

S, D, F = 2048, 576, 4608
H, DH = 32, 18
W, DIL = 8, 2
EPS = 1e-5
SCALE = DH ** -0.5
MASKED = -1000000000.0
LOG2E = 1.4426950408889634

TB = 256
NB = S // TB
HB = TB // 2
FC = 1152
HALO = 16
TOKEN_ROW = HALO + TB

f32, bf16, u32 = jnp.float32, jnp.bfloat16, jnp.uint32
NT = (((1,), (1,)), ((), ()))
D_TILES = [(k, min(128, D - k)) for k in range(0, D, 128)]
QKV_CUTS = (0, 640, 1152, 3 * D)
REST = 4


def _kernel(x_hbm, wqkv_hbm, wo_hbm, wg_hbm, wu_hbm, wd_hbm, c_hbm, wmod_hbm, out_hbm,
            x_v, wqkv_v, wo_v, wg_v, wu_v, wd_v, c_v, wmod_v,
            gate, rowvec, tmp, wqkv_t, wo_t_h2, h_a, h_b, qk_a, v_a, qk_b, v_b,
            o_v, att_t, out_v, zero, in_sems, out_sem):
    wqkv_t, wo_t_h2, h_a, h_b = (r.bitcast(bf16) for r in (wqkv_t, wo_t_h2, h_a, h_b))
    buf_a, buf_b = (qk_a, v_a), (qk_b, v_b)

    def cols(src, dst, lo, hi):
        return src.at[:, lo:hi], dst.at[:, lo:hi]

    def x_block(b):
        return x_hbm.at[:, b * TB:(b + 1) * TB], x_v.at[b]

    groups = dict(
        wq=[(c_hbm, c_v), cols(wqkv_hbm, wqkv_v, QKV_CUTS[0], QKV_CUTS[1])],
        first=[x_block(0), cols(wmod_hbm, wmod_v, 0, 640)],
        mod_a=[cols(wmod_hbm, wmod_v, 640, 2 * D)],
        wk=[cols(wqkv_hbm, wqkv_v, QKV_CUTS[1], QKV_CUTS[2])],
        wv=[cols(wqkv_hbm, wqkv_v, QKV_CUTS[2], QKV_CUTS[3])],
        x_early=[x_block(1), x_block(2)],
        x_late=[x_block(b) for b in range(3, NB)] + [(wo_hbm, wo_v)],
        mod_b=[cols(wmod_hbm, wmod_v, 2 * D, 6 * D)],
        ffn=[(wg_hbm, wg_v), (wu_hbm, wu_v), (wd_hbm, wd_v)],
    )
    copies = {name: [pltpu.make_async_copy(src, dst, in_sems.at[i]) for src, dst in group]
              for i, (name, group) in enumerate(groups.items())}
    for group in copies.values():
        for copy in group:
            copy.start()

    def wait(name):
        for copy in copies[name]:
            copy.wait()

    def prepare_wqkv(part):
        for t, (k0, kw) in enumerate(D_TILES):
            for n0 in range(QKV_CUTS[part], QKV_CUTS[part + 1], 128):
                nw = min(128, 3 * D - n0)
                tmp[t, n0:n0 + nw, 0:kw] = wqkv_v[k0:k0 + kw, n0:n0 + nw].astype(f32).T
        for t, (k0, kw) in enumerate(D_TILES):
            for d in range(DH):
                r0 = (16 * part + d if d < 16 else 48 + 2 * part + d - 16) * H
                heads = tmp[t, pl.ds(part * D + d, H, stride=DH), :]
                wqkv_t[r0:r0 + H, k0:k0 + kw] = heads[:, 0:kw].astype(bf16)

    def prepare_wo():
        for t, (n0, nw) in enumerate(D_TILES):
            tmp[t, 0:D, 0:nw] = wo_v[:, n0:n0 + nw].astype(f32)
        for t, (n0, nw) in enumerate(D_TILES):
            for tile in range(5):
                dims = range(4 * tile, 4 * tile + 4) if tile != REST else (16, 17, 16, 17)
                rows = [tmp[t, pl.ds(d, H, stride=DH), :][:, 0:nw] for d in dims]
                wo_t_h2[n0:n0 + nw, 128 * tile:128 * (tile + 1)] = (
                    jnp.concatenate(rows, axis=0).T.astype(bf16))

    def modulation(lo, hi):
        cf = c_v[...].astype(f32)
        silu = jnp.broadcast_to((cf * jax.nn.sigmoid(cf)).astype(bf16), (16, D))
        return jnp.dot(silu, wmod_v[:, lo:hi], preferred_element_type=f32)[0:8, :]

    def modulation_a():
        wait("first")
        head = modulation(0, 640)
        wait("mod_a")
        m = jnp.concatenate([head, modulation(640, 2 * D)], axis=1)
        rowvec[0, :, 0:D] = m[:, 0:D]
        rowvec[1, :, 0:D] = 1.0 + m[:, D:2 * D]

    def modulation_b():
        m = modulation(2 * D, 6 * D)
        rowvec[2, :, 0:D] = m[:, D:2 * D]
        rowvec[3, :, 0:D] = 1.0 + m[:, 2 * D:3 * D]
        for i, g in enumerate((m[:, 0:D], m[:, 3 * D:4 * D])):
            for k0, kw in D_TILES:
                gate[i, k0:k0 + kw, :] = jnp.broadcast_to(g[0:1, k0:k0 + kw], (128, kw)).T

    def norm_to_rows(xt, dst, r0, which):
        mean = jnp.sum(xt, axis=0, keepdims=True) * (1.0 / D)
        d = xt - mean
        var = jnp.sum(d * d, axis=0, keepdims=True) * (1.0 / D)
        n = d * lax.rsqrt(var + EPS)
        for k0, kw in D_TILES:
            y = (n[k0:k0 + kw, :].T * rowvec[2 * which + 1, 0:1, k0:k0 + kw]
                 + rowvec[2 * which, 0:1, k0:k0 + kw])
            dst[r0:r0 + HB, k0:k0 + kw] = y.astype(bf16)
            if kw == 128:
                last = y[HB - 8:HB, :]
        return last

    def norm_a(b, half, dst):
        return norm_to_rows(x_v[b, :, half * HB:(half + 1) * HB].astype(f32), dst, half * HB, 0)

    def residual_a(b, half):
        return x_v[b, :, half * HB:(half + 1) * HB].astype(f32) + gate[0] * att_t[2 * b + half]

    def h2(slot):
        r0 = D + slot * TB
        return wo_t_h2.at[pl.ds(r0 if isinstance(r0, int) else pl.multiple_of(r0, 16), TB)]

    def norm_b(b, half, slot):
        norm_to_rows(residual_a(b, half), h2(slot), half * HB, 1)

    def tile_ref(buf, part, t):
        return buf[1].at[t] if part == 2 else buf[0].at[5 * part + t]

    def project(parts, h, buf):
        y = lax.dot_general(h[:, 0:D], wqkv_t[512 * parts[0]:512 * (parts[-1] + 1), 0:D], NT,
                            preferred_element_type=f32)
        for i, part in enumerate(parts):
            for t in range(4):
                n0 = 512 * i + 128 * t
                tile_ref(buf, part, t)[HALO:HALO + TB, :] = y[:, n0:n0 + 128]

    def project_rest(h, buf):
        y = lax.dot_general(wqkv_t[3 * 512:3 * D, 0:D], h[:, 0:D], NT, preferred_element_type=f32)
        for part in range(3):
            yp = y[64 * part:64 * (part + 1), :]
            tile_ref(buf, part, REST)[HALO:HALO + HB, :] = jnp.concatenate(
                [yp[:, 0:HB], yp[:, HB:TB]], axis=0).T

    def low_lanes(rows):
        return lax.broadcasted_iota(jnp.int32, (rows, 128), 1) < 64

    def fill_halo(prev, buf):
        for part in (1, 2):
            for t in range(5):
                ref = tile_ref(buf, part, t)
                first = jnp.broadcast_to(ref[HALO:HALO + 1, :], (HALO, 128)) if prev is None else None
                if t != REST:
                    ref[0:HALO, :] = first if prev is None else tile_ref(prev, part, t)[TB:TB + HALO, :]
                elif prev is None:
                    ref[0:HALO, :] = jnp.where(low_lanes(HALO), first, pltpu.roll(ref[HB:HB + HALO, :], 64, 1))
                else:
                    both = jnp.where(low_lanes(HALO), ref[HB:HB + HALO, :],
                                     tile_ref(prev, part, t)[HB:HB + HALO, :])
                    ref[0:HALO, :] = pltpu.roll(both, 64, 1)

    def attend(b, buf, first_block=False, lag=2, slack=(True,), side=()):
        lane = lax.broadcasted_iota(jnp.int32, (8, 128), 1)
        low = lane < 64
        even = (lane & 32) == 0

        def taps(part, t, r, w):
            r = HALO + r - DIL * w
            return tile_ref(buf, part, t)[r:r + 8, :]

        def token(value):
            buf[0][0, pl.ds(zero[0] + TOKEN_ROW, 8), :] = value

        def products(r):
            q = [[taps(0, t, r + o, 0) for t in range(4)] for o in (0, HB)]
            q_rest = taps(0, REST, r, 0)
            out = []
            for w in range(W):
                p = []
                for half, o in enumerate((0, HB)):
                    acc = q[half][0] * taps(1, 0, r + o, w)
                    for t in range(1, 4):
                        acc = acc + q[half][t] * taps(1, t, r + o, w)
                    p.append(acc)
                out.append((jnp.where(low, p[0], p[1]) + q_rest * taps(1, REST, r, w),
                            jnp.where(low, p[1], p[0])))
                token(p[1])
            return out

        def softmax(r, partial):
            lg = [mine + pltpu.roll(other, 64, 1) for mine, other in partial]
            lg = [l + jnp.where(even, pltpu.roll(l, 96, 1), pltpu.roll(l, 32, 1)) for l in lg]
            if first_block:
                pos = lax.broadcasted_iota(jnp.int32, (8, 128), 0) + r
                lg = [jnp.where(low & (pos < DIL * w), MASKED / SCALE, l) if r < DIL * w else l
                      for w, l in enumerate(lg)]
            mx = jnp.maximum(jnp.maximum(jnp.maximum(lg[0], lg[1]), jnp.maximum(lg[2], lg[3])),
                             jnp.maximum(jnp.maximum(lg[4], lg[5]), jnp.maximum(lg[6], lg[7])))
            e = [jnp.exp2((l - mx) * (SCALE * LOG2E)) for l in lg]
            den = ((e[0] + e[1]) + (e[2] + e[3])) + ((e[4] + e[5]) + (e[6] + e[7]))
            inv = pl.reciprocal(den, approx=True)
            inv = inv * (2.0 - den * inv)
            return [x * inv for x in e]

        def combine(r, p):
            swapped = [pltpu.roll(x, 64, 1) for x in p]
            spread = [[jnp.where(low, x, y) for x, y in zip(p, swapped)],
                      [jnp.where(low, y, x) for x, y in zip(p, swapped)]]

            def weighted(weights, t, row):
                acc = weights[0] * taps(2, t, row, 0)
                for w in range(1, W):
                    acc = acc + weights[w] * taps(2, t, row, w)
                return acc

            for t in range(4):
                for half in range(2):
                    acc = weighted(spread[half], t, r + half * HB)
                    if (t, half) == (1, 1):
                        token(acc)
                    o_v[2 * b + half, r:r + 8, 128 * t:128 * (t + 1)] = acc.astype(bf16)
            acc = weighted(p, REST, r)
            o_v[2 * b, r:r + 8, 512:640] = jnp.where(low, acc, 0.0).astype(bf16)
            o_v[2 * b + 1, r:r + 8, 512:640] = jnp.where(low, 0.0, acc).astype(bf16)

        units = HB // 8
        state = {}
        for i in range(units + lag):
            for when, task in side:
                if when == i:
                    token(task())
            late = slack[i % len(slack)]
            if not late and 0 <= i - lag < units:
                combine(8 * (i - lag), state.pop(i - lag))
            if i < units:
                state[i] = products(8 * i)
            if 0 <= i - 2 < units:
                state[i - 2] = softmax(8 * (i - 2), state[i - 2])
            if late and 0 <= i - lag < units:
                combine(8 * (i - lag), state.pop(i - lag))

    def project_out(t):
        att_t[t] = lax.dot_general(wo_t_h2[0:D, :], o_v[t], NT, preferred_element_type=f32)

    def attention_stage(b, cur, nxt, h_cur, h_nxt, **kw):
        b2 = b + 2 if isinstance(b, int) else jnp.minimum(b + 2, NB - 1)
        project_rest(h_cur, nxt)
        project((1, 2), h_cur, nxt)
        project((0,), h_cur, nxt)
        attend(b, cur, side=[(1, lambda: norm_a(b2, 0, h_nxt)), (3, lambda: norm_a(b2, 1, h_nxt))], **kw)
        fill_halo(cur, nxt)

    zero[0] = 0
    wait("wq")
    prepare_wqkv(0)
    modulation_a()
    for half in range(2):
        norm_a(0, half, h_a)
    wait("wk")
    project((0,), h_a, buf_a)
    prepare_wqkv(1)
    wait("wv")
    project((1,), h_a, buf_a)
    prepare_wqkv(2)
    wait("x_early")
    project_rest(h_a, buf_a)
    project((2,), h_a, buf_a)
    for half in range(2):
        norm_a(1, half, h_b)
    fill_halo(None, buf_a)
    attention_stage(0, buf_a, buf_b, h_b, h_a, first_block=True, lag=3, slack=(False, False, True))
    wait("x_late")
    prepare_wo()

    def attention_pair(j, carry):
        b = 2 * j + 1
        project_out(b - 1)
        attention_stage(b, buf_b, buf_a, h_a, h_b)
        project_out(b)
        attention_stage(b + 1, buf_a, buf_b, h_b, h_a)
        return carry

    lax.fori_loop(0, NB // 2 - 1, attention_pair, 0)

    wait("mod_b")
    modulation_b()
    for t in range(NB - 2, 2 * NB - 2):
        project_out(t)
    attend(NB - 1, buf_b)
    for t in range(2 * NB - 2, 2 * NB):
        project_out(t)
    for half in range(2):
        norm_b(0, half, 0)
    wait("ffn")

    def out_copy(b):
        s0 = b * TB if isinstance(b, int) else pl.multiple_of(b * TB, TB)
        return pltpu.make_async_copy(out_v.at[b], out_hbm.at[:, pl.ds(s0, TB)], out_sem)

    def ffn_block(b, carry):
        nxt = jnp.minimum(b + 1, NB - 1)
        slot = b % 2
        chunks = F // FC
        acc, mid = None, {}
        for j in range(chunks + 1):
            if j < chunks:
                h = h2(slot)[:, 0:D]
                g = jnp.dot(h, wg_v[:, j * FC:(j + 1) * FC], preferred_element_type=f32)
                u = jnp.dot(h, wu_v[:, j * FC:(j + 1) * FC], preferred_element_type=f32)
                mid[j] = (g * u).astype(bf16)
            if j in (1, 2):
                norm_b(nxt, j - 1, 1 - slot)
            if j >= 1:
                y = lax.dot_general(wd_v[:, (j - 1) * FC:j * FC], mid.pop(j - 1), NT,
                                    preferred_element_type=f32)
                acc = y if acc is None else acc + y
        for half in range(2):
            lanes = slice(half * HB, (half + 1) * HB)
            out_v[b, :, lanes] = (residual_a(b, half) + gate[1] * acc[:, lanes]).astype(bf16)
        out_copy(b).start()
        return carry

    lax.fori_loop(0, NB, ffn_block, 0)
    for b in range(NB):
        out_copy(b).wait()


@jax.jit
def pallas_adaLN_cond__sliding_local_dilated__glu_gated_bilinear__prompt_kernel(
    A_x: jax.Array,
    A_wqkv: jax.Array,
    A_wo: jax.Array,
    B_x: jax.Array,
    B_w_gate: jax.Array,
    B_w_up: jax.Array,
    B_w_down: jax.Array,
    c: jax.Array,
    w_mod: jax.Array,
):
    del B_x
    vmem = pltpu.VMEM
    hbm = pl.BlockSpec(memory_space=pl.ANY)
    out_t = pl.pallas_call(
        _kernel,
        out_shape=jax.ShapeDtypeStruct((D, S), A_x.dtype),
        in_specs=[hbm] * 8,
        out_specs=hbm,
        scratch_shapes=[
            vmem((NB, D, TB), bf16),
            vmem((D, 3 * D), bf16),
            vmem((D, D), bf16),
            vmem((D, F), bf16),
            vmem((D, F), bf16),
            vmem((D, F), bf16),
            vmem((1, D), bf16),
            vmem((D, 6 * D), bf16),
            vmem((2, D, 128), f32),
            vmem((4, 8, 640), f32),
            vmem((5, 3 * D, 128), f32),
            vmem((3 * D // 2, 640), u32),
            vmem(((D + 2 * TB) // 2, 640), u32),
            vmem((TB // 2, 640), u32),
            vmem((TB // 2, 640), u32),
            vmem((10, TOKEN_ROW + 8, 128), f32),
            vmem((5, HALO + TB, 128), f32),
            vmem((10, TOKEN_ROW + 8, 128), f32),
            vmem((5, HALO + TB, 128), f32),
            vmem((2 * NB, HB, 640), bf16),
            vmem((2 * NB, D, HB), f32),
            vmem((NB, D, TB), bf16),
            pltpu.SMEM((1,), jnp.int32),
            pltpu.SemaphoreType.DMA((9,)),
            pltpu.SemaphoreType.DMA(()),
        ],
        compiler_params=pltpu.CompilerParams(vmem_limit_bytes=100 * 2**20),
    )(A_x.reshape(S, D).T, A_wqkv, A_wo, B_w_gate, B_w_up, B_w_down.T, c, w_mod)
    return out_t.T.reshape(1, S, D)
```

```python
import jax
import jax.numpy as jnp
from jax import lax
from jax.experimental import pallas as pl
from jax.experimental.pallas import tpu as pltpu

S, D, F = 2048, 576, 4608
H, DH = 32, 18
W, DIL = 8, 2
EPS = 1e-5
SCALE = DH ** -0.5
MASKED = -1000000000.0
LOG2E = 1.4426950408889634

TB = 256
NB = S // TB
HB = TB // 2
FC = 1152
HALO = 16
TOKEN_ROW = HALO + TB

f32, bf16, u32 = jnp.float32, jnp.bfloat16, jnp.uint32
NT = (((1,), (1,)), ((), ()))
D_TILES = [(k, min(128, D - k)) for k in range(0, D, 128)]
QKV_CUTS = (0, 640, 1152, 3 * D)
REST = 4


def _load_rows(ref, r0, rows, lanes, base=0):
    return pltpu.bitcast(ref[pl.ds(base + r0 // 2, rows // 2), 0:lanes], bf16)


def _store_rows(ref, r0, c0, value, base=0):
    rows, lanes = value.shape
    ref[pl.ds(base + r0 // 2, rows // 2), c0:c0 + lanes] = pltpu.bitcast(value.astype(bf16), u32)


def _kernel(x_hbm, wqkv_hbm, wo_hbm, wg_hbm, wu_hbm, wd_hbm, c_hbm, wmod_hbm, out_hbm,
            x_v, wqkv_v, wo_v, wg_v, wu_v, wd_v, c_v, wmod_v,
            gate, rowvec, tmp, wqkv_t, wo_t_h2, h_a, h_b, qk_a, v_a, qk_b, v_b,
            o_v, att_t, out_v, zero, in_sems, out_sem):
    buf_a, buf_b = (qk_a, v_a), (qk_b, v_b)

    def cols(src, dst, lo, hi):
        return src.at[:, lo:hi], dst.at[:, lo:hi]

    def x_block(b):
        return x_hbm.at[:, b * TB:(b + 1) * TB], x_v.at[b]

    groups = dict(
        wq=[(c_hbm, c_v), cols(wqkv_hbm, wqkv_v, QKV_CUTS[0], QKV_CUTS[1])],
        first=[x_block(0), cols(wmod_hbm, wmod_v, 0, 640)],
        mod_a=[cols(wmod_hbm, wmod_v, 640, 2 * D)],
        wk=[cols(wqkv_hbm, wqkv_v, QKV_CUTS[1], QKV_CUTS[2])],
        wv=[cols(wqkv_hbm, wqkv_v, QKV_CUTS[2], QKV_CUTS[3])],
        x_early=[x_block(1), x_block(2)],
        x_late=[x_block(b) for b in range(3, NB)] + [(wo_hbm, wo_v)],
        mod_b=[cols(wmod_hbm, wmod_v, 2 * D, 6 * D)],
        ffn=[(wg_hbm, wg_v), (wu_hbm, wu_v), (wd_hbm, wd_v)],
    )
    copies = {name: [pltpu.make_async_copy(src, dst, in_sems.at[i]) for src, dst in group]
              for i, (name, group) in enumerate(groups.items())}
    for group in copies.values():
        for copy in group:
            copy.start()

    def wait(name):
        for copy in copies[name]:
            copy.wait()

    def prepare_wqkv(part):
        for t, (k0, kw) in enumerate(D_TILES):
            for n0 in range(QKV_CUTS[part], QKV_CUTS[part + 1], 128):
                nw = min(128, 3 * D - n0)
                tmp[t, n0:n0 + nw, 0:kw] = wqkv_v[k0:k0 + kw, n0:n0 + nw].astype(f32).T
        for t, (k0, kw) in enumerate(D_TILES):
            for d in range(DH):
                r0 = (16 * part + d if d < 16 else 48 + 2 * part + d - 16) * H
                heads = tmp[t, pl.ds(part * D + d, H, stride=DH), :]
                _store_rows(wqkv_t, r0, k0, heads[:, 0:kw])

    def prepare_wo():
        for t, (n0, nw) in enumerate(D_TILES):
            tmp[t, 0:D, 0:nw] = wo_v[:, n0:n0 + nw].astype(f32)
        for t, (n0, nw) in enumerate(D_TILES):
            for tile in range(5):
                dims = range(4 * tile, 4 * tile + 4) if tile != REST else (16, 17, 16, 17)
                rows = [tmp[t, pl.ds(d, H, stride=DH), :][:, 0:nw] for d in dims]
                _store_rows(wo_t_h2, n0, 128 * tile, jnp.concatenate(rows, axis=0).T)

    def modulation(lo, hi):
        cf = c_v[...].astype(f32)
        silu = jnp.broadcast_to((cf * jax.nn.sigmoid(cf)).astype(bf16), (16, D))
        return jnp.dot(silu, wmod_v[:, lo:hi], preferred_element_type=f32)[0:8, :]

    def modulation_a():
        wait("first")
        head = modulation(0, 640)
        wait("mod_a")
        m = jnp.concatenate([head, modulation(640, 2 * D)], axis=1)
        rowvec[0, :, 0:D] = m[:, 0:D]
        rowvec[1, :, 0:D] = 1.0 + m[:, D:2 * D]

    def modulation_b():
        m = modulation(2 * D, 6 * D)
        rowvec[2, :, 0:D] = m[:, D:2 * D]
        rowvec[3, :, 0:D] = 1.0 + m[:, 2 * D:3 * D]
        for i, g in enumerate((m[:, 0:D], m[:, 3 * D:4 * D])):
            for k0, kw in D_TILES:
                gate[i, k0:k0 + kw, :] = jnp.broadcast_to(g[0:1, k0:k0 + kw], (128, kw)).T

    def norm_to_rows(xt, which, dst, r0, base=0):
        mean = jnp.sum(xt, axis=0, keepdims=True) * (1.0 / D)
        d = xt - mean
        var = jnp.sum(d * d, axis=0, keepdims=True) * (1.0 / D)
        n = d * lax.rsqrt(var + EPS)
        for k0, kw in D_TILES:
            y = (n[k0:k0 + kw, :].T * rowvec[2 * which + 1, 0:1, k0:k0 + kw]
                 + rowvec[2 * which, 0:1, k0:k0 + kw])
            _store_rows(dst, r0, k0, y, base)
            if kw == 128:
                last = y[HB - 8:HB, :]
        return last

    def norm_a(b, half, dst):
        return norm_to_rows(x_v[b, :, half * HB:(half + 1) * HB].astype(f32), 0, dst, half * HB)

    def residual_a(b, half):
        return x_v[b, :, half * HB:(half + 1) * HB].astype(f32) + gate[0] * att_t[2 * b + half]

    def slot_base(slot):
        base = D // 2 + slot * (TB // 2)
        return base if isinstance(base, int) else pl.multiple_of(base, 8)

    def norm_b(b, half, slot):
        norm_to_rows(residual_a(b, half), 1, wo_t_h2, half * HB, slot_base(slot))

    def tile_ref(buf, part, t):
        return buf[1].at[t] if part == 2 else buf[0].at[5 * part + t]

    def project(parts, h, buf):
        y = lax.dot_general(_load_rows(h, 0, TB, D), _load_rows(wqkv_t, 512 * parts[0], 512 * len(parts), D),
                            NT, preferred_element_type=f32)
        for i, part in enumerate(parts):
            for t in range(4):
                n0 = 512 * i + 128 * t
                tile_ref(buf, part, t)[HALO:HALO + TB, :] = y[:, n0:n0 + 128]

    def project_rest(h, buf):
        y = lax.dot_general(_load_rows(wqkv_t, 3 * 512, 3 * 64, D), _load_rows(h, 0, TB, D),
                            NT, preferred_element_type=f32)
        for part in range(3):
            yp = y[64 * part:64 * (part + 1), :]
            tile_ref(buf, part, REST)[HALO:HALO + HB, :] = jnp.concatenate(
                [yp[:, 0:HB], yp[:, HB:TB]], axis=0).T

    def low_lanes(rows):
        return lax.broadcasted_iota(jnp.int32, (rows, 128), 1) < 64

    def fill_halo(prev, buf):
        for part in (1, 2):
            for t in range(5):
                ref = tile_ref(buf, part, t)
                first = jnp.broadcast_to(ref[HALO:HALO + 1, :], (HALO, 128)) if prev is None else None
                if t != REST:
                    ref[0:HALO, :] = first if prev is None else tile_ref(prev, part, t)[TB:TB + HALO, :]
                elif prev is None:
                    ref[0:HALO, :] = jnp.where(low_lanes(HALO), first, pltpu.roll(ref[HB:HB + HALO, :], 64, 1))
                else:
                    both = jnp.where(low_lanes(HALO), ref[HB:HB + HALO, :],
                                     tile_ref(prev, part, t)[HB:HB + HALO, :])
                    ref[0:HALO, :] = pltpu.roll(both, 64, 1)

    def attend(b, buf, first_block=False, lag=2, slack=(True,), side=()):
        lane = lax.broadcasted_iota(jnp.int32, (8, 128), 1)
        low = lane < 64
        even = (lane & 32) == 0

        def taps(part, t, r, w):
            r = HALO + r - DIL * w
            return tile_ref(buf, part, t)[r:r + 8, :]

        def token(value):
            buf[0][0, pl.ds(zero[0] + TOKEN_ROW, 8), :] = value

        def products(r):
            q = [[taps(0, t, r + o, 0) for t in range(4)] for o in (0, HB)]
            q_rest = taps(0, REST, r, 0)
            out = []
            for w in range(W):
                p = []
                for half, o in enumerate((0, HB)):
                    acc = q[half][0] * taps(1, 0, r + o, w)
                    for t in range(1, 4):
                        acc = acc + q[half][t] * taps(1, t, r + o, w)
                    p.append(acc)
                out.append((jnp.where(low, p[0], p[1]) + q_rest * taps(1, REST, r, w),
                            jnp.where(low, p[1], p[0])))
                token(p[1])
            return out

        def softmax(r, partial):
            lg = [mine + pltpu.roll(other, 64, 1) for mine, other in partial]
            lg = [l + jnp.where(even, pltpu.roll(l, 96, 1), pltpu.roll(l, 32, 1)) for l in lg]
            if first_block:
                pos = lax.broadcasted_iota(jnp.int32, (8, 128), 0) + r
                lg = [jnp.where(low & (pos < DIL * w), MASKED / SCALE, l) if r < DIL * w else l
                      for w, l in enumerate(lg)]
            mx = jnp.maximum(jnp.maximum(jnp.maximum(lg[0], lg[1]), jnp.maximum(lg[2], lg[3])),
                             jnp.maximum(jnp.maximum(lg[4], lg[5]), jnp.maximum(lg[6], lg[7])))
            e = [jnp.exp2((l - mx) * (SCALE * LOG2E)) for l in lg]
            den = ((e[0] + e[1]) + (e[2] + e[3])) + ((e[4] + e[5]) + (e[6] + e[7]))
            inv = pl.reciprocal(den, approx=True)
            inv = inv * (2.0 - den * inv)
            return [x * inv for x in e]

        def combine(r, p):
            swapped = [pltpu.roll(x, 64, 1) for x in p]
            spread = [[jnp.where(low, x, y) for x, y in zip(p, swapped)],
                      [jnp.where(low, y, x) for x, y in zip(p, swapped)]]

            def weighted(weights, t, row):
                acc = weights[0] * taps(2, t, row, 0)
                for w in range(1, W):
                    acc = acc + weights[w] * taps(2, t, row, w)
                return acc

            for t in range(4):
                for half in range(2):
                    acc = weighted(spread[half], t, r + half * HB)
                    if (t, half) == (1, 1):
                        token(acc)
                    o_v[2 * b + half, r:r + 8, 128 * t:128 * (t + 1)] = acc.astype(bf16)
            acc = weighted(p, REST, r)
            o_v[2 * b, r:r + 8, 512:640] = jnp.where(low, acc, 0.0).astype(bf16)
            o_v[2 * b + 1, r:r + 8, 512:640] = jnp.where(low, 0.0, acc).astype(bf16)

        units = HB // 8
        state = {}
        for i in range(units + lag):
            for when, task in side:
                if when == i:
                    token(task())
            late = slack[i % len(slack)]
            if not late and 0 <= i - lag < units:
                combine(8 * (i - lag), state.pop(i - lag))
            if i < units:
                state[i] = products(8 * i)
            if 0 <= i - 2 < units:
                state[i - 2] = softmax(8 * (i - 2), state[i - 2])
            if late and 0 <= i - lag < units:
                combine(8 * (i - lag), state.pop(i - lag))

    def project_out(t):
        att_t[t] = lax.dot_general(_load_rows(wo_t_h2, 0, D, 640), o_v[t], NT, preferred_element_type=f32)

    def attention_stage(b, cur, nxt, h_cur, h_nxt, **kw):
        b2 = b + 2 if isinstance(b, int) else jnp.minimum(b + 2, NB - 1)
        project_rest(h_cur, nxt)
        project((1, 2), h_cur, nxt)
        project((0,), h_cur, nxt)
        attend(b, cur, side=[(1, lambda: norm_a(b2, 0, h_nxt)), (3, lambda: norm_a(b2, 1, h_nxt))], **kw)
        fill_halo(cur, nxt)

    zero[0] = 0
    wait("wq")
    prepare_wqkv(0)
    modulation_a()
    for half in range(2):
        norm_a(0, half, h_a)
    wait("wk")
    project((0,), h_a, buf_a)
    prepare_wqkv(1)
    wait("wv")
    project((1,), h_a, buf_a)
    prepare_wqkv(2)
    wait("x_early")
    project_rest(h_a, buf_a)
    project((2,), h_a, buf_a)
    for half in range(2):
        norm_a(1, half, h_b)
    fill_halo(None, buf_a)
    attention_stage(0, buf_a, buf_b, h_b, h_a, first_block=True, lag=3, slack=(False, False, True))
    wait("x_late")
    prepare_wo()

    def attention_pair(j, carry):
        b = 2 * j + 1
        project_out(b - 1)
        attention_stage(b, buf_b, buf_a, h_a, h_b)
        project_out(b)
        attention_stage(b + 1, buf_a, buf_b, h_b, h_a)
        return carry

    lax.fori_loop(0, NB // 2 - 1, attention_pair, 0)

    wait("mod_b")
    modulation_b()
    for t in range(NB - 2, 2 * NB - 2):
        project_out(t)
    attend(NB - 1, buf_b)
    for t in range(2 * NB - 2, 2 * NB):
        project_out(t)
    for half in range(2):
        norm_b(0, half, 0)
    wait("ffn")

    def out_copy(b):
        s0 = b * TB if isinstance(b, int) else pl.multiple_of(b * TB, TB)
        return pltpu.make_async_copy(out_v.at[b], out_hbm.at[:, pl.ds(s0, TB)], out_sem)

    def ffn_block(b, carry):
        nxt = jnp.minimum(b + 1, NB - 1)
        slot = b % 2
        chunks = F // FC
        acc, mid = None, {}
        for j in range(chunks + 1):
            if j < chunks:
                h = _load_rows(wo_t_h2, 0, TB, D, slot_base(slot))
                g = jnp.dot(h, wg_v[:, j * FC:(j + 1) * FC], preferred_element_type=f32)
                u = jnp.dot(h, wu_v[:, j * FC:(j + 1) * FC], preferred_element_type=f32)
                mid[j] = (g * u).astype(bf16)
            if j in (1, 2):
                norm_b(nxt, j - 1, 1 - slot)
            if j >= 1:
                y = lax.dot_general(wd_v[:, (j - 1) * FC:j * FC], mid.pop(j - 1), NT,
                                    preferred_element_type=f32)
                acc = y if acc is None else acc + y
        for half in range(2):
            lanes = slice(half * HB, (half + 1) * HB)
            out_v[b, :, lanes] = (residual_a(b, half) + gate[1] * acc[:, lanes]).astype(bf16)
        out_copy(b).start()
        return carry

    lax.fori_loop(0, NB, ffn_block, 0)
    for b in range(NB):
        out_copy(b).wait()


@jax.jit
def pallas_adaLN_cond__sliding_local_dilated__glu_gated_bilinear__prompt_kernel(
    A_x: jax.Array,
    A_wqkv: jax.Array,
    A_wo: jax.Array,
    B_x: jax.Array,
    B_w_gate: jax.Array,
    B_w_up: jax.Array,
    B_w_down: jax.Array,
    c: jax.Array,
    w_mod: jax.Array,
):
    del B_x
    vmem = pltpu.VMEM
    hbm = pl.BlockSpec(memory_space=pl.ANY)
    out_t = pl.pallas_call(
        _kernel,
        out_shape=jax.ShapeDtypeStruct((D, S), A_x.dtype),
        in_specs=[hbm] * 8,
        out_specs=hbm,
        scratch_shapes=[
            vmem((NB, D, TB), bf16),
            vmem((D, 3 * D), bf16),
            vmem((D, D), bf16),
            vmem((D, F), bf16),
            vmem((D, F), bf16),
            vmem((D, F), bf16),
            vmem((1, D), bf16),
            vmem((D, 6 * D), bf16),
            vmem((2, D, 128), f32),
            vmem((4, 8, 640), f32),
            vmem((5, 3 * D, 128), f32),
            vmem((3 * D // 2, 640), u32),
            vmem(((D + 2 * TB) // 2, 640), u32),
            vmem((TB // 2, 640), u32),
            vmem((TB // 2, 640), u32),
            vmem((10, TOKEN_ROW + 8, 128), f32),
            vmem((5, HALO + TB, 128), f32),
            vmem((10, TOKEN_ROW + 8, 128), f32),
            vmem((5, HALO + TB, 128), f32),
            vmem((2 * NB, HB, 640), bf16),
            vmem((2 * NB, D, HB), f32),
            vmem((NB, D, TB), bf16),
            pltpu.SMEM((1,), jnp.int32),
            pltpu.SemaphoreType.DMA((9,)),
            pltpu.SemaphoreType.DMA(()),
        ],
        compiler_params=pltpu.CompilerParams(vmem_limit_bytes=100 * 2**20),
    )(A_x.reshape(S, D).T, A_wqkv, A_wo, B_w_gate, B_w_up, B_w_down.T, c, w_mod)
    return out_t.T.reshape(1, S, D)
```

```python
import jax
import jax.numpy as jnp
from jax import lax
from jax.experimental import pallas as pl
from jax.experimental.pallas import tpu as pltpu

S, D, F = 2048, 576, 4608
H, DH = 32, 18
W, DIL = 8, 2
EPS = 1e-5
SCALE = DH ** -0.5
MASKED = -1000000000.0
LOG2E = 1.4426950408889634

TB = 256
NB = S // TB
HB = TB // 2
FC = 1152
HALO = 16
TOKEN_ROW = HALO + TB

f32, bf16, u32 = jnp.float32, jnp.bfloat16, jnp.uint32
NT = (((1,), (1,)), ((), ()))
D_TILES = [(k, min(128, D - k)) for k in range(0, D, 128)]
QKV_CUTS = (0, 640, 1152, 3 * D)
REST = 4


def _load_rows(ref, r0, rows, lanes, base=0):
    return pltpu.bitcast(ref[pl.ds(base + r0 // 2, rows // 2), 0:lanes], bf16)


def _store_rows(ref, r0, c0, value, base=0):
    rows, lanes = value.shape
    ref[pl.ds(base + r0 // 2, rows // 2), c0:c0 + lanes] = pltpu.bitcast(value.astype(bf16), u32)


def _kernel(x_hbm, wqkv_hbm, wo_hbm, wg_hbm, wu_hbm, wd_hbm, c_hbm, wmod_hbm, out_hbm,
            x_v, wqkv_v, wo_v, wg_v, wu_v, wd_v, c_v, wmod_v,
            gate, rowvec, tmp, wqkv_t, wo_t_h2, h_a, h_b, qk_a, v_a, qk_b, v_b,
            o_v, att_t, out_v, zero, in_sems, out_sem):
    buf_a, buf_b = (qk_a, v_a), (qk_b, v_b)

    def cols(src, dst, lo, hi):
        return src.at[:, lo:hi], dst.at[:, lo:hi]

    def x_block(b):
        return x_hbm.at[:, b * TB:(b + 1) * TB], x_v.at[b]

    groups = dict(
        wq=[(c_hbm, c_v), cols(wqkv_hbm, wqkv_v, QKV_CUTS[0], QKV_CUTS[1])],
        first=[x_block(0), cols(wmod_hbm, wmod_v, 0, 640)],
        mod_a=[cols(wmod_hbm, wmod_v, 640, 2 * D)],
        wk=[cols(wqkv_hbm, wqkv_v, QKV_CUTS[1], QKV_CUTS[2])],
        wv=[cols(wqkv_hbm, wqkv_v, QKV_CUTS[2], QKV_CUTS[3])],
        x_early=[x_block(1), x_block(2)],
        x_late=[x_block(b) for b in range(3, NB)] + [(wo_hbm, wo_v)],
        mod_b=[cols(wmod_hbm, wmod_v, 2 * D, 6 * D)],
        ffn=[(wg_hbm, wg_v), (wu_hbm, wu_v), (wd_hbm, wd_v)],
    )
    copies = {name: [pltpu.make_async_copy(src, dst, in_sems.at[i]) for src, dst in group]
              for i, (name, group) in enumerate(groups.items())}
    for group in copies.values():
        for copy in group:
            copy.start()

    def wait(name):
        for copy in copies[name]:
            copy.wait()

    def prepare_wqkv(part):
        for t, (k0, kw) in enumerate(D_TILES):
            for n0 in range(QKV_CUTS[part], QKV_CUTS[part + 1], 128):
                nw = min(128, 3 * D - n0)
                tmp[t, n0:n0 + nw, 0:kw] = wqkv_v[k0:k0 + kw, n0:n0 + nw].astype(f32).T
        for t, (k0, kw) in enumerate(D_TILES):
            for d in range(DH):
                r0 = (16 * part + d if d < 16 else 48 + 2 * part + d - 16) * H
                heads = tmp[t, pl.ds(part * D + d, H, stride=DH), :]
                _store_rows(wqkv_t, r0, k0, heads[:, 0:kw])

    def prepare_wo():
        for t, (n0, nw) in enumerate(D_TILES):
            tmp[t, 0:D, 0:nw] = wo_v[:, n0:n0 + nw].astype(f32)
        for t, (n0, nw) in enumerate(D_TILES):
            for tile in range(5):
                dims = range(4 * tile, 4 * tile + 4) if tile != REST else (16, 17, 16, 17)
                rows = [tmp[t, pl.ds(d, H, stride=DH), :][:, 0:nw] for d in dims]
                _store_rows(wo_t_h2, n0, 128 * tile, jnp.concatenate(rows, axis=0).T)

    def modulation(lo, hi):
        cf = c_v[...].astype(f32)
        silu = jnp.broadcast_to((cf * jax.nn.sigmoid(cf)).astype(bf16), (16, D))
        return jnp.dot(silu, wmod_v[:, lo:hi], preferred_element_type=f32)[0:8, :]

    def modulation_a():
        wait("first")
        head = modulation(0, 640)
        wait("mod_a")
        m = jnp.concatenate([head, modulation(640, 2 * D)], axis=1)
        rowvec[0, :, 0:D] = m[:, 0:D]
        rowvec[1, :, 0:D] = 1.0 + m[:, D:2 * D]

    def modulation_b():
        m = modulation(2 * D, 6 * D)
        rowvec[2, :, 0:D] = m[:, D:2 * D]
        rowvec[3, :, 0:D] = 1.0 + m[:, 2 * D:3 * D]
        for i, g in enumerate((m[:, 0:D], m[:, 3 * D:4 * D])):
            for k0, kw in D_TILES:
                gate[i, k0:k0 + kw, :] = jnp.broadcast_to(g[0:1, k0:k0 + kw], (128, kw)).T

    def norm_to_rows(xt, which, dst, r0, base=0):
        mean = jnp.sum(xt, axis=0, keepdims=True) * (1.0 / D)
        d = xt - mean
        var = jnp.sum(d * d, axis=0, keepdims=True) * (1.0 / D)
        n = d * lax.rsqrt(var + EPS)
        for k0, kw in D_TILES:
            y = (n[k0:k0 + kw, :].T * rowvec[2 * which + 1, 0:1, k0:k0 + kw]
                 + rowvec[2 * which, 0:1, k0:k0 + kw])
            _store_rows(dst, r0, k0, y, base)
            if kw == 128:
                last = y[HB - 8:HB, :]
        return last

    def norm_a(b, half, dst):
        return norm_to_rows(x_v[b, :, half * HB:(half + 1) * HB].astype(f32), 0, dst, half * HB)

    def residual_a(b, half):
        return x_v[b, :, half * HB:(half + 1) * HB].astype(f32) + gate[0] * att_t[2 * b + half]

    def slot_base(slot):
        base = D // 2 + slot * (TB // 2)
        return base if isinstance(base, int) else pl.multiple_of(base, 8)

    def norm_b(b, half, slot):
        norm_to_rows(residual_a(b, half), 1, wo_t_h2, half * HB, slot_base(slot))

    def tile_ref(buf, part, t):
        return buf[1].at[t] if part == 2 else buf[0].at[5 * part + t]

    def project(part, h, buf):
        y = lax.dot_general(_load_rows(h, 0, TB, D), _load_rows(wqkv_t, 512 * part, 512, D),
                            NT, preferred_element_type=f32)
        for t in range(4):
            tile_ref(buf, part, t)[HALO:HALO + TB, :] = y[:, 128 * t:128 * (t + 1)]

    def project_rest(h, buf):
        y = lax.dot_general(_load_rows(wqkv_t, 3 * 512, 3 * 64, D), _load_rows(h, 0, TB, D),
                            NT, preferred_element_type=f32)
        for part in range(3):
            yp = y[64 * part:64 * (part + 1), :]
            tile_ref(buf, part, REST)[HALO:HALO + HB, :] = jnp.concatenate(
                [yp[:, 0:HB], yp[:, HB:TB]], axis=0).T

    def low_lanes(rows):
        return lax.broadcasted_iota(jnp.int32, (rows, 128), 1) < 64

    def fill_halo(prev, buf):
        for part in (1, 2):
            for t in range(5):
                ref = tile_ref(buf, part, t)
                first = jnp.broadcast_to(ref[HALO:HALO + 1, :], (HALO, 128)) if prev is None else None
                if t != REST:
                    ref[0:HALO, :] = first if prev is None else tile_ref(prev, part, t)[TB:TB + HALO, :]
                elif prev is None:
                    ref[0:HALO, :] = jnp.where(low_lanes(HALO), first, pltpu.roll(ref[HB:HB + HALO, :], 64, 1))
                else:
                    both = jnp.where(low_lanes(HALO), ref[HB:HB + HALO, :],
                                     tile_ref(prev, part, t)[HB:HB + HALO, :])
                    ref[0:HALO, :] = pltpu.roll(both, 64, 1)

    def attend(b, buf, first_block=False, side=None):
        lane = lax.broadcasted_iota(jnp.int32, (8, 128), 1)
        low = lane < 64
        even = (lane & 32) == 0

        def taps(part, t, r, w):
            r = HALO + r - DIL * w
            return tile_ref(buf, part, t)[r:r + 8, :]

        def token(value):
            buf[0][0, pl.ds(zero[0] + TOKEN_ROW, 8), :] = value

        def products(r):
            q = [[taps(0, t, r + o, 0) for t in range(4)] for o in (0, HB)]
            q_rest = taps(0, REST, r, 0)
            out = []
            for w in range(W):
                p = []
                for half, o in enumerate((0, HB)):
                    acc = q[half][0] * taps(1, 0, r + o, w)
                    for t in range(1, 4):
                        acc = acc + q[half][t] * taps(1, t, r + o, w)
                    p.append(acc)
                out.append((jnp.where(low, p[0], p[1]) + q_rest * taps(1, REST, r, w),
                            jnp.where(low, p[1], p[0])))
                token(p[0])
            return out

        def softmax(r, partial):
            lg = [mine + pltpu.roll(other, 64, 1) for mine, other in partial]
            lg = [l + jnp.where(even, pltpu.roll(l, 96, 1), pltpu.roll(l, 32, 1)) for l in lg]
            if first_block:
                pos = lax.broadcasted_iota(jnp.int32, (8, 128), 0) + r
                lg = [jnp.where(low & (pos < DIL * w), MASKED / SCALE, l) if r < DIL * w else l
                      for w, l in enumerate(lg)]
            mx = jnp.maximum(jnp.maximum(jnp.maximum(lg[0], lg[1]), jnp.maximum(lg[2], lg[3])),
                             jnp.maximum(jnp.maximum(lg[4], lg[5]), jnp.maximum(lg[6], lg[7])))
            e = [jnp.exp2((l - mx) * (SCALE * LOG2E)) for l in lg]
            den = ((e[0] + e[1]) + (e[2] + e[3])) + ((e[4] + e[5]) + (e[6] + e[7]))
            inv = pl.reciprocal(den, approx=True)
            inv = inv * (2.0 - den * inv)
            return [x * inv for x in e]

        def combine(r, p):
            swapped = [pltpu.roll(x, 64, 1) for x in p]
            spread = [[jnp.where(low, x, y) for x, y in zip(p, swapped)],
                      [jnp.where(low, y, x) for x, y in zip(p, swapped)]]

            def weighted(weights, t, row):
                acc = weights[0] * taps(2, t, row, 0)
                for w in range(1, W):
                    acc = acc + weights[w] * taps(2, t, row, w)
                return acc

            for t in range(4):
                for half in range(2):
                    acc = weighted(spread[half], t, r + half * HB)
                    if (t, half) == (1, 1):
                        token(acc)
                    o_v[2 * b + half, r:r + 8, 128 * t:128 * (t + 1)] = acc.astype(bf16)
            acc = weighted(p, REST, r)
            o_v[2 * b, r:r + 8, 512:640] = jnp.where(low, acc, 0.0).astype(bf16)
            o_v[2 * b + 1, r:r + 8, 512:640] = jnp.where(low, 0.0, acc).astype(bf16)

        units = HB // 8
        partial, weights = {}, {}
        for i in range(units + 2):
            if side and i in side:
                token(side[i]())
            if i < units:
                partial[i] = products(8 * i)
            if 1 <= i <= units:
                weights[i - 1] = softmax(8 * (i - 1), partial.pop(i - 1))
            if i >= 2:
                combine(8 * (i - 2), weights.pop(i - 2))

    def project_out(t):
        att_t[t] = lax.dot_general(_load_rows(wo_t_h2, 0, D, 640), o_v[t], NT, preferred_element_type=f32)

    def attention_stage(b, cur, nxt, h_cur, h_nxt, first_block=False):
        b2 = b + 2 if isinstance(b, int) else jnp.minimum(b + 2, NB - 1)
        project_rest(h_cur, nxt)
        for part in range(3):
            project(part, h_cur, nxt)
        attend(b, cur, first_block,
               side={1: lambda: norm_a(b2, 0, h_nxt), 3: lambda: norm_a(b2, 1, h_nxt)})
        fill_halo(cur, nxt)

    zero[0] = 0
    tmp[4] = jnp.zeros(tmp.shape[1:], f32)
    wait("wq")
    prepare_wqkv(0)
    modulation_a()
    for half in range(2):
        norm_a(0, half, h_a)
    wait("wk")
    project(0, h_a, buf_a)
    prepare_wqkv(1)
    wait("wv")
    project(1, h_a, buf_a)
    prepare_wqkv(2)
    wait("x_early")
    project_rest(h_a, buf_a)
    project(2, h_a, buf_a)
    for half in range(2):
        norm_a(1, half, h_b)
    fill_halo(None, buf_a)
    attention_stage(0, buf_a, buf_b, h_b, h_a, first_block=True)
    wait("x_late")
    prepare_wo()

    def attention_pair(j, carry):
        b = 2 * j + 1
        project_out(b - 1)
        attention_stage(b, buf_b, buf_a, h_a, h_b)
        project_out(b)
        attention_stage(b + 1, buf_a, buf_b, h_b, h_a)
        return carry

    lax.fori_loop(0, NB // 2 - 1, attention_pair, 0)

    wait("mod_b")
    modulation_b()
    for t in range(NB - 2, 2 * NB - 2):
        project_out(t)
    attend(NB - 1, buf_b)
    for t in range(2 * NB - 2, 2 * NB):
        project_out(t)
    for half in range(2):
        norm_b(0, half, 0)
    wait("ffn")

    def out_copy(b):
        s0 = b * TB if isinstance(b, int) else pl.multiple_of(b * TB, TB)
        return pltpu.make_async_copy(out_v.at[b], out_hbm.at[:, pl.ds(s0, TB)], out_sem)

    def ffn_block(b, carry):
        nxt = jnp.minimum(b + 1, NB - 1)
        slot = b % 2
        chunks = F // FC
        acc, mid = None, {}
        for j in range(chunks + 1):
            if j < chunks:
                h = _load_rows(wo_t_h2, 0, TB, D, slot_base(slot))
                g = jnp.dot(h, wg_v[:, j * FC:(j + 1) * FC], preferred_element_type=f32)
                u = jnp.dot(h, wu_v[:, j * FC:(j + 1) * FC], preferred_element_type=f32)
                mid[j] = (g * u).astype(bf16)
            if j in (1, 2):
                norm_b(nxt, j - 1, 1 - slot)
            if j >= 1:
                y = lax.dot_general(wd_v[:, (j - 1) * FC:j * FC], mid.pop(j - 1), NT,
                                    preferred_element_type=f32)
                acc = y if acc is None else acc + y
        for half in range(2):
            lanes = slice(half * HB, (half + 1) * HB)
            out_v[b, :, lanes] = (residual_a(b, half) + gate[1] * acc[:, lanes]).astype(bf16)
        out_copy(b).start()
        return carry

    lax.fori_loop(0, NB, ffn_block, 0)
    for b in range(NB):
        out_copy(b).wait()


@jax.jit
def pallas_adaLN_cond__sliding_local_dilated__glu_gated_bilinear__prompt_kernel(
    A_x: jax.Array,
    A_wqkv: jax.Array,
    A_wo: jax.Array,
    B_x: jax.Array,
    B_w_gate: jax.Array,
    B_w_up: jax.Array,
    B_w_down: jax.Array,
    c: jax.Array,
    w_mod: jax.Array,
):
    del B_x
    vmem = pltpu.VMEM
    hbm = pl.BlockSpec(memory_space=pl.ANY)
    out_t = pl.pallas_call(
        _kernel,
        out_shape=jax.ShapeDtypeStruct((D, S), A_x.dtype),
        in_specs=[hbm] * 8,
        out_specs=hbm,
        scratch_shapes=[
            vmem((NB, D, TB), bf16),
            vmem((D, 3 * D), bf16),
            vmem((D, D), bf16),
            vmem((D, F), bf16),
            vmem((D, F), bf16),
            vmem((D, F), bf16),
            vmem((1, D), bf16),
            vmem((D, 6 * D), bf16),
            vmem((2, D, 128), f32),
            vmem((4, 8, 640), f32),
            vmem((5, 3 * D + 24, 128), f32),
            vmem((3 * D // 2, 640), u32),
            vmem(((D + 2 * TB) // 2, 640), u32),
            vmem((TB // 2, 640), u32),
            vmem((TB // 2, 640), u32),
            vmem((10, TOKEN_ROW + 8, 128), f32),
            vmem((5, HALO + TB, 128), f32),
            vmem((10, TOKEN_ROW + 8, 128), f32),
            vmem((5, HALO + TB, 128), f32),
            vmem((2 * NB, HB, 640), bf16),
            vmem((2 * NB, D, HB), f32),
            vmem((NB, D, TB), bf16),
            pltpu.SMEM((1,), jnp.int32),
            pltpu.SemaphoreType.DMA((9,)),
            pltpu.SemaphoreType.DMA(()),
        ],
        compiler_params=pltpu.CompilerParams(vmem_limit_bytes=100 * 2**20),
    )(A_x.reshape(S, D).T, A_wqkv, A_wo, B_w_gate, B_w_up, B_w_down.T, c, w_mod)
    return out_t.T.reshape(1, S, D)
```
